```python
import jax
import jax.numpy as jnp

def _softmax(x, axis=-1):
    return jax.nn.softmax(x, axis=axis)

def _gelu(x):
    return jax.nn.gelu(x, approximate=True)

def _silu(x):
    return jax.nn.silu(x)

def _sigmoid(x):
    return jax.nn.sigmoid(x)

def _layernorm(x, axis=-1, eps=1e-05):
    m = jnp.mean(x, axis=axis, keepdims=True)
    v = jnp.var(x, axis=axis, keepdims=True)
    return (x - m) / jnp.sqrt(v + eps)

def _scatter_add(tgt, idx, src, axis=0):
    return tgt.at[idx].add(src)

def _segment_sum(src, seg, n):
    return jax.ops.segment_sum(src, seg, n)

class _Rng:

    def __init__(self, key):
        self._k = key

    def _next(self):
        self._k, sub = jax.random.split(self._k)
        return sub

    def normal(self, shape):
        return jax.random.normal(self._next(), shape, dtype=jnp.bfloat16)

    def randint(self, lo, hi, shape):
        return jax.random.randint(self._next(), shape, lo, hi, dtype=jnp.int32)

    def uniform(self, shape, lo=0.0, hi=1.0):
        return jax.random.uniform(self._next(), shape, jnp.bfloat16, lo, hi)

    def permutation(self, n):
        return jax.random.permutation(self._next(), n)
kernel_name = 'interleave_layers__memory_aug_infini_attn__mixer_s_mlp__prompt'

def setup_inputs():
    _rng = _Rng(jax.random.key(int.from_bytes(__import__("os").urandom(4), "little")))
    _w = lambda a: (lambda t: t.astype(jnp.bfloat16) if jnp.issubdtype(t.dtype, jnp.floating) else t)(jnp.asarray(a))

    def _A_setup():
        B, S, D, H = (1, 2048, 1024, 32)
        N = 4
        L = max(1, S // N)
        sc = D ** (-0.5)
        return {'x': _w((lambda *s: _rng.normal(s) * 0.05)(B, N * L, D)), 'wq': _w((lambda *s: _rng.normal(s) * 0.05)(D, D) * sc), 'wk': _w((lambda *s: _rng.normal(s) * 0.05)(D, D) * sc), 'wv': _w((lambda *s: _rng.normal(s) * 0.05)(D, D) * sc), 'wo': _w((lambda *s: _rng.normal(s) * 0.05)(D, D) * sc), 'beta': _w((lambda *s: _rng.normal(s) * 0.05)(H))}
    _A_in = _A_setup()

    def _B_setup():
        B, S, D, F = (1, 2048, 1024, 3584)
        return {'x': _w((lambda *s: _rng.normal(s) * 0.05)(B, S, D)), 'w1': _w((lambda *s: _rng.normal(s) * 0.05)(D, D) * D ** (-0.5)), 'w2': _w((lambda *s: _rng.normal(s) * 0.05)(D, D) * D ** (-0.5)), 'w3': _w((lambda *s: _rng.normal(s) * 0.05)(D, F) * D ** (-0.5)), 'w4': _w((lambda *s: _rng.normal(s) * 0.05)(F, D) * F ** (-0.5))}
    _B_in = _B_setup()
    return {'A_x': _A_in['x'], 'A_wq': _A_in['wq'], 'A_wk': _A_in['wk'], 'A_wv': _A_in['wv'], 'A_wo': _A_in['wo'], 'A_beta': _A_in['beta'], 'B_x': _B_in['x'], 'B_w1': _B_in['w1'], 'B_w2': _B_in['w2'], 'B_w3': _B_in['w3'], 'B_w4': _B_in['w4']}

def reference(A_x, A_wq, A_wk, A_wv, A_wo, A_beta, B_x, B_w1, B_w2, B_w3, B_w4):

    def _A_ref(x, wq, wk, wv, wo, beta):
        B, S, D = x.shape
        H = 32
        Dh = D // H
        N = 4
        L = S // N
        q = (lambda x, *d: x.transpose(*d))((x @ wq).reshape(B, S, H, Dh), 0, 2, 1, 3).reshape(B, H, N, L, Dh)
        k = (lambda x, *d: x.transpose(*d))((x @ wk).reshape(B, S, H, Dh), 0, 2, 1, 3).reshape(B, H, N, L, Dh)
        v = (lambda x, *d: x.transpose(*d))((x @ wv).reshape(B, S, H, Dh), 0, 2, 1, 3).reshape(B, H, N, L, Dh)
        phi = lambda t: jnp.where(t > 0, t + 1.0, jnp.exp(t))
        scale = Dh ** (-0.5)
        ar = jnp.arange(L)
        mask = (lambda x, dt: x.astype(dt))(ar[:, None] < ar[None, :], x.dtype) * -1000000000.0
        g = _sigmoid(beta).reshape(1, H, 1, 1)
        M = jnp.einsum('bhd,bhe->bhde', q[:, :, 0, 0, :] * 0.0, q[:, :, 0, 0, :] * 0.0)
        z = q[:, :, 0, 0, :] * 0.0
        outs = []
        for s in range(N):
            qs, ks, vs = (q[:, :, s].copy(), k[:, :, s].copy(), v[:, :, s].copy())
            logits = jnp.einsum('bhqd,bhkd->bhqk', qs, ks) * scale + mask
            p = _softmax(logits, axis=-1)
            a_dot = jnp.einsum('bhqk,bhkd->bhqd', p, vs)
            pq = phi(qs)
            num = jnp.einsum('bhld,bhde->bhle', pq, M)
            den = jnp.einsum('bhld,bhd->bhl', pq, z)[..., None] + 1e-06
            a_mem = num / den
            o = g * a_mem + (1.0 - g) * a_dot
            outs.append(o)
            pk = phi(ks)
            M = M + jnp.einsum('bhld,bhle->bhde', pk, vs)
            z = z + jnp.einsum('bhld->bhd', pk)
        o = (lambda x, *d: x.transpose(*d))(jnp.stack(outs, 2).reshape(B, H, S, Dh), 0, 2, 1, 3).reshape(B, S, D)
        return o @ wo

    def _B_ref(x, w1, w2, w3, w4):
        B, S, D = x.shape
        h = _gelu(_layernorm(x, axis=-1) @ w1)
        c = D // 4
        g0 = jnp.pad(h[:, :, 0 * c:1 * c], ((0, 0), (1, 0), (0, 0)))[:, :S, :]
        g1 = jnp.pad(h[:, :, 1 * c:2 * c], ((0, 0), (0, 1), (0, 0)))[:, 1:, :]
        g2 = jnp.pad(h[:, :, 2 * c:3 * c], ((0, 0), (2, 0), (0, 0)))[:, :S, :]
        g3 = jnp.pad(h[:, :, 3 * c:], ((0, 0), (0, 2), (0, 0)))[:, 2:, :]
        hs = jnp.concatenate([g0, g1, g2, g3], axis=-1) @ w2
        x1 = x + hs
        h2 = _gelu(_layernorm(x1, axis=-1) @ w3) @ w4
        return x1 + h2
    x = A_x
    x = x + _A_ref(_layernorm(x, axis=-1), A_wq, A_wk, A_wv, A_wo, A_beta)
    x = x + _B_ref(_layernorm(x, axis=-1), B_w1, B_w2, B_w3, B_w4)
    x = x + _A_ref(_layernorm(x, axis=-1), A_wq, A_wk, A_wv, A_wo, A_beta)
    x = x + _B_ref(_layernorm(x, axis=-1), B_w1, B_w2, B_w3, B_w4)
    return x
```

```python
import functools
import math

import numpy as np
import jax
import jax.numpy as jnp
from jax import lax
import jax.experimental.pallas as pl
import jax.experimental.pallas.tpu as pltpu

S_LEN = 2048
D = 1024
F = 3584
H = 32
DH = 32
NSEG = 4
L = 512
G = 8
NU = NSEG * G
OFF = (0, 128, 384, 768)
EPS = 1e-5
QSCALE = float(DH ** -0.5 * math.log2(math.e))
NEG = -1e30
BM = 256
NB = S_LEN // BM

f32 = jnp.float32
bf16 = jnp.bfloat16
i32 = jnp.int32
NT = (((1,), (1,)), ((), ()))


def i2b(x):
    return pltpu.bitcast(x, bf16)


def b2i(x):
    return pltpu.bitcast(x, i32)


def _ln(x):
    m = jnp.mean(x, axis=-1, keepdims=True)
    d = x - m
    v = jnp.mean(d * d, axis=-1, keepdims=True)
    return d * lax.rsqrt(v + EPS)


def _gelu(x):
    c0 = math.sqrt(2.0 / math.pi)
    c1 = c0 * 0.044715
    return (0.5 * x) * (1.0 + jnp.tanh(x * (c0 + c1 * (x * x))))


def _phi(t):
    return jnp.where(t > 0, t + 1.0, jnp.exp(t))


def _dot(a, b):
    return jnp.dot(a, b, preferred_element_type=f32)


def _kernel(x_hbm, wq_hbm, wk_hbm, wv_hbm, wo_hbm, beta_ref, w1_hbm, w2_hbm, w3_hbm, w4_hbm,
            out_hbm,
            xio, wq, wk, wv, wo, w1, w2, w3, w4,
            xf, zf, xn, qs, kb, pq, pk, vt, sb, pb, mb, rb, ob, mt, hb, y1b, gt,
            sem_x, sem_w, sem_o):
    win = [(wq_hbm, wq), (wk_hbm, wk), (wv_hbm, wv), (wo_hbm, wo),
           (w1_hbm, w1), (w2_hbm, w2), (w3_hbm, w3), (w4_hbm, w4)]

    def w_copy(i):
        return pltpu.make_async_copy(win[i][0], win[i][1], sem_w.at[i])

    def x_copy(i):
        return pltpu.make_async_copy(x_hbm.at[pl.ds(i * BM, BM)], xio.at[pl.ds(i * BM, BM)], sem_x.at[i])

    def o_copy(i):
        r = pl.multiple_of(i * BM, BM)
        return pltpu.make_async_copy(xio.at[pl.ds(r, BM)], out_hbm.at[pl.ds(r, BM)], sem_o.at[i])

    for i in range(NB):
        x_copy(i).start()
    for i in range(3):
        w_copy(i).start()

    gt[...] = jax.nn.sigmoid(beta_ref[...])
    hb[0:8, :] = jnp.zeros((8, D), f32)
    hb[8 + S_LEN:16 + S_LEN, :] = jnp.zeros((8, D), f32)

    for i in range(NB):
        x_copy(i).wait()
    def init_body(i, c):
        r = pl.multiple_of(i * BM, BM)
        x = xio[pl.ds(r, BM), :].astype(f32)
        xf[pl.ds(r, BM), :] = x
        xn[pl.ds(pl.multiple_of(i * (BM // 2), BM // 2), BM // 2), :] = b2i(_ln(x).astype(bf16))
        return c
    lax.fori_loop(0, NB, init_body, 0)

    def unit(u):
        return u // G, u % G

    def xs_of(s):
        return i2b(xn[pl.ds(pl.multiple_of(s * (L // 2), L // 2), L // 2), :])

    def col(g):
        return pl.ds(pl.multiple_of(g * 128, 128), 128)

    def D1qk(u):
        s, g = unit(u)
        xs = xs_of(s)
        q = _dot(xs, wq[:, col(g)])
        qs[...] = b2i((q * QSCALE).astype(bf16))
        pq[u % 4] = b2i(_phi(q).astype(bf16))
        k = _dot(xs, wk[:, col(g)])
        kb[...] = b2i(k.astype(bf16))
        pk[u % 4] = b2i(_phi(k).astype(bf16))

    def D1v(u):
        s, g = unit(u)
        v = _dot(xs_of(s), wv[:, col(g)])
        vt[...] = b2i(v.astype(bf16).T)

    def S_stage(j):
        n = 128 * (j + 1)
        lane = lax.broadcasted_iota(i32, (64, 128), 1)
        hm = [jnp.where((lane >= 32 * h) & (lane < 32 * h + 32), -1, 0).astype(i32) for h in range(4)]
        valid = lax.broadcasted_iota(i32, (128, 128), 0) <= lax.broadcasted_iota(i32, (128, 128), 1)
        k4 = i2b(kb[:n // 2, :])
        qj = qs[64 * j:64 * j + 64, :]
        qst = i2b(jnp.concatenate([qj & hm[h] for h in range(4)], axis=0))
        sT = lax.dot_general(k4, qst, NT, preferred_element_type=f32)
        for h in range(4):
            sh = sT[:, 128 * h:128 * h + 128]
            dg = jnp.where(valid, sh[128 * j:], NEG)
            sh = jnp.concatenate([sh[:128 * j], dg], axis=0) if j else dg
            sb[OFF[j]:OFF[j] + n, 128 * h:128 * h + 128] = sh
            m = jnp.max(sh, axis=0, keepdims=True)
            mb[8 * j:8 * j + 8, 128 * h:128 * h + 128] = jnp.broadcast_to(m, (8, 128))

    def E_stage(j):
        for h in range(4):
            m = mb[8 * j:8 * j + 8, 128 * h:128 * h + 128]
            l = None
            for i in range(j + 1):
                r0 = OFF[j] + 128 * i
                s = sb[r0:r0 + 128, 128 * h:128 * h + 128]
                p = jnp.exp2(s.reshape(16, 8, 128) - m[None])
                li = jnp.sum(p, axis=0)
                l = li if l is None else l + li
                pb[r0 // 2:r0 // 2 + 64, 128 * h:128 * h + 128] = b2i(p.reshape(128, 128).astype(bf16))
            lt = jnp.sum(l, axis=0, keepdims=True)
            rb[8 * j:8 * j + 8, 128 * h:128 * h + 128] = jnp.broadcast_to(1.0 / lt, (8, 128))

    def V_dots(j):
        n = 128 * (j + 1)
        outs = []
        for h in range(4):
            vh = i2b(vt[16 * h:16 * h + 16, :n])
            p = i2b(pb[OFF[j] // 2:(OFF[j] + n) // 2, 128 * h:128 * h + 128])
            oT = _dot(vh, p)
            r = rb[8 * j:8 * j + 8, 128 * h:128 * h + 128]
            outs.append((oT.reshape(4, 8, 128) * r[None]).reshape(32, 128))
        return jnp.concatenate(outs, axis=0)

    def V_finish(u, adots, first_seg, update):
        s, g = unit(u)
        adot = jnp.concatenate(adots, axis=1)
        gate = gt[pl.ds(pl.multiple_of(g * 32, 32), 32), :]
        gate = jnp.concatenate(
            [jnp.broadcast_to(gate[8 * h:8 * h + 8][None], (4, 8, 128)).reshape(32, 128) for h in range(4)], axis=0)
        gate = jnp.concatenate([gate] * 4, axis=1)
        if first_seg:
            o = (1.0 - gate) * adot
        else:
            mtb = mt[g].astype(bf16)
            nd = lax.dot_general(mtb, i2b(pq[u % 4]), NT, preferred_element_type=f32)
            num = nd[:128]
            den = jnp.concatenate(
                [jnp.broadcast_to(nd[128 + h:129 + h], (32, 512)) for h in range(4)], axis=0) + 1e-6
            o = gate * (num / den) + (1.0 - gate) * adot
        ob[pl.ds(pl.multiple_of(s * 256, 256), 256), col(g)] = b2i(o.astype(bf16).T)
        if update:
            ones = jnp.full((8, 512), 0x3F803F80, i32)
            lhs = i2b(jnp.concatenate([vt[...], ones], axis=0))
            upd = _dot(lhs, i2b(pk[u % 4]))
            r = lax.broadcasted_iota(i32, (144, 128), 0)
            c = lax.broadcasted_iota(i32, (144, 128), 1)
            rh = jnp.where(r < 128, r // 32, r - 128)
            upd = jnp.where(rh == c // 32, upd, 0.0)
            if first_seg:
                mt[g] = upd
            else:
                mt[g] = mt[g] + upd

    def D2(v):
        s, c = unit(v)
        o = i2b(ob[pl.ds(pl.multiple_of(s * 256, 256), 256), :])
        y = _dot(o, wo[:, col(c)])
        rows = pl.ds(pl.multiple_of(s * L, L), L)
        xf[rows, col(c)] = xf[rows, col(c)] + y

    def a_iter(t, do_qk, do_s, do_e, do_v, do_d2, first_seg=False, update=True):
        adots = []
        for j in range(4):
            if do_v:
                adots.append(V_dots(j))
            if do_e:
                E_stage(j)
            if do_s:
                S_stage(j)
            if j == 0 and do_v:
                pass
            if j == 1 and do_d2:
                D2(t - 9)
        if do_v:
            V_finish(t - 1, adots, first_seg, update)
        if do_qk:
            D1qk(t + 2)
        if do_e:
            D1v(t)

    def lnln(i):
        r = pl.multiple_of(i * BM, BM)
        z = _ln(xf[pl.ds(r, BM), :])
        zf[pl.ds(r, BM), :] = z
        y1b[...] = b2i(_ln(z).astype(bf16))

    def ba_body(i, c):
        hh = _gelu(_dot(i2b(y1b[...]), w1[...]))
        hb[pl.ds(pl.multiple_of(i * BM + 8, 8), BM), :] = hh
        lnln(jnp.minimum(i + 1, NB - 1))
        return c

    def shifted(r0):
        win_ = hb[pl.ds(pl.multiple_of(r0, 8), 144), :]
        parts = []
        for gi, sh in enumerate((-1, 1, -2, 2)):
            parts.append(win_[8 + sh:8 + sh + 128, 256 * gi:256 * gi + 256])
        return jnp.concatenate(parts, axis=1).astype(bf16)

    def bb_body(i, rep):
        rows = [pl.multiple_of(i * BM + 128 * a, 128) for a in range(2)]
        x1 = [zf[pl.ds(r, 128), :] + _dot(shifted(r), w2[...]) for r in rows]
        y2 = [_ln(v).astype(bf16) for v in x1]
        gg = [None, None]
        gg[0] = _gelu(_dot(y2[0], w3[...])).astype(bf16)
        gg[1] = _gelu(_dot(y2[1], w3[...])).astype(bf16)
        for a in range(2):
            r = rows[a]
            xo = xf[pl.ds(r, 128), :] + x1[a] + _dot(gg[a], w4[...])
            xf[pl.ds(r, 128), :] = xo
            xn[pl.ds(pl.multiple_of(r // 2, 64), 64), :] = b2i(_ln(xo).astype(bf16))
            xio[pl.ds(r, 128), :] = xo.astype(bf16)

        @pl.when(rep == 1)
        def _():
            o_copy(i).start()
        return rep

    def rep_body(rep, c):
        @pl.when(rep == 0)
        def _():
            for i in range(3):
                w_copy(i).wait()
            for i in range(3, 8):
                w_copy(i).start()
        a_iter(-2, True, False, False, False, False)
        a_iter(-1, True, True, False, False, False)
        a_iter(0, True, True, True, False, False)

        def l1(t, c):
            a_iter(t, True, True, True, True, False, first_seg=True)
            return c
        lax.fori_loop(1, 9, l1, 0)

        @pl.when(rep == 0)
        def _():
            w_copy(3).wait()

        def l2(t, c):
            a_iter(t, True, True, True, True, True)
            return c
        lax.fori_loop(9, 30, l2, 0)
        a_iter(30, False, True, True, True, True, update=False)
        a_iter(31, False, False, True, True, True, update=False)
        a_iter(32, False, False, False, True, True, update=False)

        def l3(t, c):
            D2(t - 9)
            return c
        lax.fori_loop(33, 41, l3, 0)

        @pl.when(rep == 0)
        def _():
            for i in range(4, 8):
                w_copy(i).wait()
        lnln(0)
        lax.fori_loop(0, NB, ba_body, 0)
        lax.fori_loop(0, NB, bb_body, rep)
        return c

    lax.fori_loop(0, 2, rep_body, 0)
    for i in range(NB):
        o_copy(i).wait()


def build(name="infini_mixer"):
    vm = pltpu.VMEM
    scratch = [
        vm((S_LEN, D), bf16),
        vm((D, D), bf16), vm((D, D), bf16), vm((D, D), bf16), vm((D, D), bf16),
        vm((D, D), bf16), vm((D, D), bf16), vm((D, F), bf16), vm((F, D), bf16),
        vm((S_LEN, D), f32),
        vm((S_LEN, D), f32),
        vm((S_LEN // 2, D), i32),
        vm((256, 128), i32), vm((256, 128), i32),
        vm((4, 256, 128), i32), vm((4, 256, 128), i32),
        vm((64, 512), i32),
        vm((1280, 512), f32), vm((640, 512), i32),
        vm((32, 512), f32), vm((32, 512), f32),
        vm((S_LEN // 2, D), i32),
        vm((G, 144, 128), f32),
        vm((S_LEN + 16, D), f32),
        vm((BM // 2, D), i32),
        vm((H * 8, 128), f32),
        pltpu.SemaphoreType.DMA((NB,)), pltpu.SemaphoreType.DMA((8,)), pltpu.SemaphoreType.DMA((NB,)),
    ]
    any_spec = pl.BlockSpec(memory_space=pl.ANY)
    return pl.pallas_call(
        _kernel,
        out_shape=jax.ShapeDtypeStruct((S_LEN, D), bf16),
        in_specs=[any_spec] * 5 + [pl.BlockSpec(memory_space=pltpu.VMEM)] + [any_spec] * 4,
        out_specs=any_spec,
        scratch_shapes=scratch,
        compiler_params=pltpu.CompilerParams(vmem_limit_bytes=110 * 2 ** 20),
        name=name,
    )


@jax.jit
def pallas_interleave_layers__memory_aug_infini_attn__mixer_s_mlp__prompt_kernel(A_x, A_wq, A_wk, A_wv, A_wo, A_beta, B_x, B_w1, B_w2, B_w3, B_w4):
    beta = jnp.broadcast_to(A_beta.astype(f32).reshape(H, 1, 1), (H, 8, 128)).reshape(H * 8, 128)
    out = build()(A_x.reshape(S_LEN, D), A_wq, A_wk, A_wv, A_wo, beta, B_w1, B_w2, B_w3, B_w4)
    return out.reshape(1, S_LEN, D)
```

```python
import functools
import math

import numpy as np
import jax
import jax.numpy as jnp
from jax import lax
import jax.experimental.pallas as pl
import jax.experimental.pallas.tpu as pltpu

S_LEN = 2048
D = 1024
F = 3584
H = 32
DH = 32
NSEG = 4
L = 512
G = 8
NU = NSEG * G
OFF = (0, 128, 384, 768)
EPS = 1e-5
QSCALE = float(DH ** -0.5 * math.log2(math.e))
NEG = -1e30
BM = 256
NB = S_LEN // BM

f32 = jnp.float32
bf16 = jnp.bfloat16
i32 = jnp.int32
NT = (((1,), (1,)), ((), ()))

CFG = dict(
    order="V0 E0 S0 X V1 E1 S1 D N V2 E2 S2 R V3 F U E3 S3 W Q K",
    mode="full",
    scopes=False,
)


def i2b(x):
    return pltpu.bitcast(x, bf16)


def b2i(x):
    return pltpu.bitcast(x, i32)


def _ln(x):
    m = jnp.mean(x, axis=-1, keepdims=True)
    d = x - m
    v = jnp.mean(d * d, axis=-1, keepdims=True)
    return d * lax.rsqrt(v + EPS)


def _ln2(x):
    m = jnp.mean(x, axis=-1, keepdims=True)
    d = x - m
    v = jnp.mean(d * d, axis=-1, keepdims=True)
    r = lax.rsqrt(v + EPS)
    r2 = r * lax.rsqrt(v * r * r + EPS)
    return d * r, d * r2


def _gelu(x):
    c0 = math.sqrt(2.0 / math.pi)
    c1 = c0 * 0.044715
    return (0.5 * x) * (1.0 + jnp.tanh(x * (c0 + c1 * (x * x))))


def _phi(t):
    return jnp.where(t > 0, t + 1.0, jnp.exp(t))


def _dot(a, b):
    return jnp.dot(a, b, preferred_element_type=f32)


class _NoScope:
    def __enter__(self):
        return self

    def __exit__(self, *a):
        return False


def _kernel(x_hbm, wq_hbm, wk_hbm, wv_hbm, wo_hbm, beta_ref, w1_hbm, w2_hbm, w3_hbm, w4_hbm,
            out_hbm,
            xio, wq, wk, wv, wo, w1, w2, w3, w4,
            xf, zf, xn, y1, qs, kb, pq, pk, vt, sb, pb, mb, rb, ob, mt, hb, gt,
            sem_x, sem_q, sem_w, sem_o, *, cfg):
    scope = jax.named_scope if cfg["scopes"] else (lambda name: _NoScope())
    wlate = [(wo_hbm, wo), (w1_hbm, w1), (w2_hbm, w2), (w3_hbm, w3), (w4_hbm, w4)]
    wqkv = [(wq_hbm, wq), (wk_hbm, wk), (wv_hbm, wv)]

    def w_copy(i):
        return pltpu.make_async_copy(wlate[i][0], wlate[i][1], sem_w.at[i])

    def qkv_copy(m, q):
        cols = pl.ds(256 * q, 256)
        return pltpu.make_async_copy(wqkv[m][0].at[:, cols], wqkv[m][1].at[:, cols], sem_q.at[m, q])

    def x_copy(i):
        return pltpu.make_async_copy(x_hbm.at[pl.ds(i * L, L)], xio.at[pl.ds(i * L, L)], sem_x.at[i])

    def o_copy(i):
        r = pl.multiple_of(i * BM, BM)
        return pltpu.make_async_copy(xio.at[pl.ds(r, BM)], out_hbm.at[pl.ds(r, BM)], sem_o.at[i])

    x_copy(0).start()
    qkv_copy(0, 0).start()
    qkv_copy(1, 0).start()
    x_copy(1).start()
    qkv_copy(2, 0).start()

    gt[...] = jax.nn.sigmoid(beta_ref[...])
    hb[0:8, :] = jnp.zeros((8, D), f32)
    hb[8 + S_LEN:16 + S_LEN, :] = jnp.zeros((8, D), f32)
    pb[...] = jnp.zeros(pb.shape, i32)
    rb[...] = jnp.zeros(rb.shape, f32)
    vt[...] = jnp.zeros(vt.shape, i32)
    pk[3] = jnp.zeros(pk.shape[1:], i32)

    def unit(u):
        return u // G, u % G

    def xs_of(s):
        return i2b(xn[pl.ds(pl.multiple_of(s * (L // 2), L // 2), L // 2), :])

    def col(g):
        return pl.ds(pl.multiple_of(g * 128, 128), 128)

    def rows64(c):
        return pl.ds(pl.multiple_of(c * 64, 64), 64), pl.ds(pl.multiple_of(c * 32, 32), 32)

    def XN(c, rep):
        r, rp = rows64(c)
        x = jnp.where(rep == 0, xio[r, :].astype(f32), xf[r, :])
        xf[r, :] = x
        xn[rp, :] = b2i(_ln(x).astype(bf16))

    def LNLN(c):
        r, rp = rows64(c)
        z, y = _ln2(xf[r, :])
        zf[r, :] = z
        y1[rp, :] = b2i(y.astype(bf16))

    def D1q(u):
        s, g = unit(u)
        q = _dot(xs_of(s), wq[:, col(g)])
        qs[...] = b2i((q * QSCALE).astype(bf16))
        pq[u % 4] = b2i(_phi(q).astype(bf16))

    def D1k(u):
        s, g = unit(u)
        k = _dot(xs_of(s), wk[:, col(g)])
        kb[...] = b2i(k.astype(bf16))
        pk[u % 4] = b2i(_phi(k).astype(bf16))

    def D1v(u):
        s, g = unit(u)
        v = _dot(xs_of(s), wv[:, col(g)])
        vt[...] = b2i(v.astype(bf16).T)

    def S_stage(j):
        n = 128 * (j + 1)
        lane = lax.broadcasted_iota(i32, (64, 128), 1)
        hm = [jnp.where((lane >= 32 * h) & (lane < 32 * h + 32), -1, 0).astype(i32) for h in range(4)]
        valid = lax.broadcasted_iota(i32, (128, 128), 0) <= lax.broadcasted_iota(i32, (128, 128), 1)
        k4 = i2b(kb[:n // 2, :])
        qj = qs[64 * j:64 * j + 64, :]
        qst = i2b(jnp.concatenate([qj & hm[h] for h in range(4)], axis=0))
        sT = lax.dot_general(k4, qst, NT, preferred_element_type=f32)
        for h in range(4):
            sh = sT[:, 128 * h:128 * h + 128]
            dg = jnp.where(valid, sh[128 * j:], NEG)
            sh = jnp.concatenate([sh[:128 * j], dg], axis=0) if j else dg
            sb[OFF[j]:OFF[j] + n, 128 * h:128 * h + 128] = sh
            m = jnp.max(sh, axis=0, keepdims=True)
            mb[8 * j:8 * j + 8, 128 * h:128 * h + 128] = jnp.broadcast_to(m, (8, 128))

    def E_stage(j):
        for h in range(4):
            m = mb[8 * j:8 * j + 8, 128 * h:128 * h + 128]
            l = None
            for i in range(j + 1):
                r0 = OFF[j] + 128 * i
                s = sb[r0:r0 + 128, 128 * h:128 * h + 128]
                p = jnp.exp2(s.reshape(16, 8, 128) - m[None])
                li = jnp.sum(p, axis=0)
                l = li if l is None else l + li
                pb[r0 // 2:r0 // 2 + 64, 128 * h:128 * h + 128] = b2i(p.reshape(128, 128).astype(bf16))
            lt = jnp.sum(l, axis=0, keepdims=True)
            rb[8 * j:8 * j + 8, 128 * h:128 * h + 128] = jnp.broadcast_to(1.0 / lt, (8, 128))

    def V_dots(j):
        n = 128 * (j + 1)
        outs = []
        for h in range(4):
            vh = i2b(vt[16 * h:16 * h + 16, :n])
            p = i2b(pb[OFF[j] // 2:(OFF[j] + n) // 2, 128 * h:128 * h + 128])
            oT = _dot(vh, p)
            r = rb[8 * j:8 * j + 8, 128 * h:128 * h + 128]
            outs.append((oT.reshape(4, 8, 128) * r[None]).reshape(32, 128))
        return jnp.concatenate(outs, axis=0)

    def gate_of(g):
        gate = gt[pl.ds(pl.multiple_of(g * 32, 32), 32), :]
        return jnp.concatenate(
            [jnp.broadcast_to(gate[8 * h:8 * h + 8][None], (4, 8, 128)).reshape(32, 128) for h in range(4)], axis=0)

    def M_read(u):
        s, g = unit(u)
        mtb = mt[g].astype(bf16)
        nd = lax.dot_general(mtb, i2b(pq[u % 4]), NT, preferred_element_type=f32)
        num = nd[:128]
        den = jnp.concatenate(
            [jnp.broadcast_to(nd[128 + h:129 + h], (32, 512)) for h in range(4)], axis=0) + 1e-6
        return num / den

    def V_finish(u, adots, amem):
        s, g = unit(u)
        adot = jnp.concatenate(adots, axis=1)
        gate = jnp.concatenate([gate_of(g)] * 4, axis=1)
        o = (1.0 - gate) * adot
        if amem is not None:
            o = gate * amem + o
        ob[pl.ds(pl.multiple_of(s * 256, 256), 256), col(g)] = b2i(o.astype(bf16).T)

    def M_update(u, first_seg):
        s, g = unit(u)
        ones = jnp.full((8, 512), 0x3F803F80, i32)
        lhs = i2b(jnp.concatenate([vt[...], ones], axis=0))
        upd = _dot(lhs, i2b(pk[u % 4]))
        r = lax.broadcasted_iota(i32, (144, 128), 0)
        c = lax.broadcasted_iota(i32, (144, 128), 1)
        rh = jnp.where(r < 128, r // 32, r - 128)
        upd = jnp.where(rh == c // 32, upd, 0.0)
        if first_seg:
            mt[g] = upd
        else:
            mt[g] = mt[g] + upd

    def D2(v):
        s, c = unit(v)
        o = i2b(ob[pl.ds(pl.multiple_of(s * 256, 256), 256), :])
        y = _dot(o, wo[:, col(c)])
        rows = pl.ds(pl.multiple_of(s * L, L), L)
        xf[rows, col(c)] = xf[rows, col(c)] + y

    def a_iter(t, rep, on, first_seg=False):
        adots = [None] * 4
        amem = None
        uv = jnp.maximum(t - 1, 0)
        for tok in cfg["order"].split():
            k = tok[0]
            if k not in on:
                continue
            if k == "V":
                adots[int(tok[1])] = V_dots(int(tok[1]))
            elif k == "E":
                E_stage(int(tok[1]))
            elif k == "S":
                S_stage(int(tok[1]))
            elif k == "D":
                D2(t - 9)
            elif k == "X":
                XN(jnp.minimum(t + 10, 31), rep)
            elif k == "N":
                LNLN(jnp.maximum(t - 17, 0))
            elif k == "R":
                if not first_seg:
                    amem = M_read(uv)
            elif k == "F":
                V_finish(uv, adots, amem)
            elif k == "U":
                M_update(uv, first_seg)
            elif k == "Q":
                D1q(jnp.minimum(t + 2, NU - 1))
            elif k == "K":
                D1k(jnp.minimum(t + 2, NU - 1))
            elif k == "W":
                D1v(t)

    def ba_body(i, c):
        lhs = i2b(y1[pl.ds(pl.multiple_of(i * (BM // 2), BM // 2), BM // 2), :])
        hb[pl.ds(pl.multiple_of(i * BM + 8, 8), BM), :] = _gelu(_dot(lhs, w1[...]))
        return c

    def shifted(r0):
        win_ = hb[pl.ds(pl.multiple_of(r0, 8), 144), :]
        parts = []
        for gi, sh in enumerate((-1, 1, -2, 2)):
            parts.append(win_[8 + sh:8 + sh + 128, 256 * gi:256 * gi + 256])
        return jnp.concatenate(parts, axis=1).astype(bf16)

    def bb_body(i, rep):
        rows = [pl.multiple_of(i * BM + 128 * a, 128) for a in range(2)]
        x1 = [zf[pl.ds(r, 128), :] + _dot(shifted(r), w2[...]) for r in rows]
        y2 = [_ln(v).astype(bf16) for v in x1]
        gg = [_gelu(_dot(y2[a], w3[...])).astype(bf16) for a in range(2)]
        for a in range(2):
            r = rows[a]
            xo = xf[pl.ds(r, 128), :] + x1[a] + _dot(gg[a], w4[...])
            xf[pl.ds(r, 128), :] = xo
            xio[pl.ds(r, 128), :] = xo.astype(bf16)

        @pl.when(rep == 1)
        def _():
            o_copy(i).start()
        return rep

    ALL = "VESDXNRFUQKW"

    def l1(t, rep):
        for tt, wi in ((2, 0), (4, 1), (6, 2)):
            @pl.when((rep == 0) & (t == tt))
            def _():
                w_copy(wi).start()
        for tt, q in ((2, 2), (4, 3)):
            @pl.when((rep == 0) & (t == tt))
            def _():
                for m in range(3):
                    qkv_copy(m, q).wait()

        @pl.when((rep == 0) & (t == 6))
        def _():
            x_copy(2).wait()
        a_iter(t, rep, "VESXRFUQKW", first_seg=True)
        return rep

    def l2(t, rep):
        for tt, wi in ((11, 3), (16, 4)):
            @pl.when((rep == 0) & (t == tt))
            def _():
                w_copy(wi).start()

        @pl.when((rep == 0) & (t == 14))
        def _():
            x_copy(3).wait()
        a_iter(t, rep, ALL)
        return rep

    if cfg["mode"] == "l2":
        lax.fori_loop(9, 30, l2, 0)
        return
    if cfg["mode"] == "bb":
        lax.fori_loop(0, NB, bb_body, 0)
        return

    def rep_body(rep, c):
        with scope("z_xn0"):
            @pl.when(rep == 0)
            def _():
                x_copy(0).wait()

            def xn0(c_, carry):
                XN(c_, rep)
                return carry
            lax.fori_loop(0, 8, xn0, 0)

        with scope("z_apro"):
            @pl.when(rep == 0)
            def _():
                qkv_copy(0, 0).wait()
                qkv_copy(1, 0).wait()
            a_iter(-2, rep, "QK")

            @pl.when(rep == 0)
            def _():
                x_copy(1).wait()
                qkv_copy(2, 0).wait()
                for m in range(3):
                    qkv_copy(m, 1).start()
            XN(8, rep)
            XN(9, rep)
            a_iter(-1, rep, "SQK")

            @pl.when(rep == 0)
            def _():
                for m in range(3):
                    qkv_copy(m, 1).wait()
                for q in (2, 3):
                    for m in range(3):
                        qkv_copy(m, q).start()
                x_copy(2).start()
                x_copy(3).start()

        with scope("z_l1"):
            lax.fori_loop(0, 9, l1, rep)

        @pl.when(rep == 0)
        def _():
            w_copy(0).wait()

        with scope("z_l2"):
            lax.fori_loop(9, 30, l2, rep)
        with scope("z_aepi"):
            a_iter(30, rep, "VESDNRFW")
            a_iter(31, rep, "VEDNRFW")
            a_iter(32, rep, "VDNRF")

        def l3(t, c):
            a_iter(t, rep, "DN")
            return c
        with scope("z_l3"):
            lax.fori_loop(33, 41, l3, 0)

        @pl.when(rep == 0)
        def _():
            for i in range(1, 5):
                w_copy(i).wait()

        def ln3(c_, carry):
            LNLN(c_)
            return carry
        with scope("z_ln3"):
            lax.fori_loop(24, 32, ln3, 0)
        with scope("z_ba"):
            lax.fori_loop(0, NB, ba_body, 0)
        with scope("z_bb"):
            lax.fori_loop(0, NB, bb_body, rep)
        return c

    lax.fori_loop(0, 2, rep_body, 0)
    with scope("z_owait"):
        for i in range(NB):
            o_copy(i).wait()


def build(cfg, name="infini_mixer"):
    vm = pltpu.VMEM
    scratch = [
        vm((S_LEN, D), bf16),
        vm((D, D), bf16), vm((D, D), bf16), vm((D, D), bf16), vm((D, D), bf16),
        vm((D, D), bf16), vm((D, D), bf16), vm((D, F), bf16), vm((F, D), bf16),
        vm((S_LEN, D), f32),
        vm((S_LEN, D), f32),
        vm((S_LEN // 2, D), i32),
        vm((S_LEN // 2, D), i32),
        vm((256, 128), i32), vm((256, 128), i32),
        vm((4, 256, 128), i32), vm((4, 256, 128), i32),
        vm((64, 512), i32),
        vm((1280, 512), f32), vm((640, 512), i32),
        vm((32, 512), f32), vm((32, 512), f32),
        vm((S_LEN // 2, D), i32),
        vm((G, 144, 128), f32),
        vm((S_LEN + 16, D), f32),
        vm((H * 8, 128), f32),
        pltpu.SemaphoreType.DMA((4,)), pltpu.SemaphoreType.DMA((3, 4)),
        pltpu.SemaphoreType.DMA((5,)), pltpu.SemaphoreType.DMA((NB,)),
    ]
    any_spec = pl.BlockSpec(memory_space=pl.ANY)
    return pl.pallas_call(
        functools.partial(_kernel, cfg=cfg),
        out_shape=jax.ShapeDtypeStruct((S_LEN, D), bf16),
        in_specs=[any_spec] * 5 + [pl.BlockSpec(memory_space=pltpu.VMEM)] + [any_spec] * 4,
        out_specs=any_spec,
        scratch_shapes=scratch,
        compiler_params=pltpu.CompilerParams(vmem_limit_bytes=110 * 2 ** 20),
        name=name,
    )


def make_kernel(cfg, name="infini_mixer"):
    def pallas_interleave_layers__memory_aug_infini_attn__mixer_s_mlp__prompt_kernel(A_x, A_wq, A_wk, A_wv, A_wo, A_beta, B_x, B_w1, B_w2, B_w3, B_w4):
        beta = jnp.broadcast_to(A_beta.astype(f32).reshape(H, 1, 1), (H, 8, 128)).reshape(H * 8, 128)
        out = build(cfg, name)(A_x.reshape(S_LEN, D), A_wq, A_wk, A_wv, A_wo, beta, B_w1, B_w2, B_w3, B_w4)
        return out.reshape(1, S_LEN, D)
    return jax.jit(kernel)


kernel = make_kernel(CFG)
```

```python
import functools
import math

import numpy as np
import jax
import jax.numpy as jnp
from jax import lax
import jax.experimental.pallas as pl
import jax.experimental.pallas.tpu as pltpu

S_LEN = 2048
D = 1024
F = 3584
H = 32
DH = 32
NSEG = 4
L = 512
G = 8
NU = NSEG * G
OFF = (0, 128, 384, 768)
EPS = 1e-5
QSCALE = float(DH ** -0.5 * math.log2(math.e))
NEG = -1e30
BM = 256
NB = S_LEN // BM

f32 = jnp.float32
bf16 = jnp.bfloat16
i32 = jnp.int32
NT = (((1,), (1,)), ((), ()))

CONSTRAINTS = [("V.", "E#"), ("E.", "S#"), ("V.", "W"), ("U", "W"), ("S.", "Q"), ("S.", "K"), ("R", "U"), ("V.", "F"), ("R", "F")]
SEARCH_MODE = "A"
SEARCH_T = 400.0


def score(loops, total):
    rep, xn0, l1, l2, l3, ln3 = loops[:6]
    ln = lambda x: x[1] - x[0]
    straight = ln(rep) - ln(xn0) - ln(l1) - ln(l2) - ln(l3) - ln(ln3)
    parts = [ln(xn0), ln(l1), ln(l2), ln(l3), ln(ln3), straight]
    return 4 * ln(xn0) + 9 * ln(l1) + 21 * ln(l2) + 8 * ln(l3) + 4 * ln(ln3) + straight, parts


CFG = dict(
    order1="V0 E0 S0 V1 E1 S1 D V2 E2 R V3 S2 U E3 S3 N W Q X K F",
    order2="V0 V1 E0 S0 X R E1 D N V2 E2 S1 S2 V3 U F E3 S3 W K Q",
    order3="V0 E0 S0 V1 N V2 R E2 E1 V3 U E3 S2 S3 S1 W X F Q D K",
    mode="full",
    scopes=False,
)


def i2b(x):
    return pltpu.bitcast(x, bf16)


def b2i(x):
    return pltpu.bitcast(x, i32)


def _ln(x):
    m = jnp.mean(x, axis=-1, keepdims=True)
    d = x - m
    v = jnp.mean(d * d, axis=-1, keepdims=True)
    return d * lax.rsqrt(v + EPS)


def _ln2(x):
    m = jnp.mean(x, axis=-1, keepdims=True)
    d = x - m
    v = jnp.mean(d * d, axis=-1, keepdims=True)
    r = lax.rsqrt(v + EPS)
    r2 = r * lax.rsqrt(v * r * r + EPS)
    return d * r, d * r2


def _gelu(x):
    c0 = math.sqrt(2.0 / math.pi)
    c1 = c0 * 0.044715
    return (0.5 * x) * (1.0 + jnp.tanh(x * (c0 + c1 * (x * x))))


def _phi(t):
    return jnp.where(t > 0, t + 1.0, jnp.exp(t))


def _dot(a, b):
    return jnp.dot(a, b, preferred_element_type=f32)


class _NoScope:
    def __enter__(self):
        return self

    def __exit__(self, *a):
        return False


def _kernel(x_hbm, wq_hbm, wk_hbm, wv_hbm, wo_hbm, beta_ref, w1_hbm, w2_hbm, w3_hbm, w4_hbm,
            out_hbm,
            xio, wq, wk, wv, wo, w1, w2, w3, w4,
            xf, zf, xn, y1, qs, kb, pq, pk, vt, sb, pb, mb, rb, ob, mt, hb, gt,
            sem_x, sem_q, sem_w, sem_o, *, cfg):
    scope = jax.named_scope if cfg["scopes"] else (lambda name: _NoScope())
    wlate = [(wo_hbm, wo), (w1_hbm, w1), (w2_hbm, w2), (w3_hbm, w3), (w4_hbm, w4)]
    wqkv = [(wq_hbm, wq), (wk_hbm, wk), (wv_hbm, wv)]

    def w_copy(i):
        return pltpu.make_async_copy(wlate[i][0], wlate[i][1], sem_w.at[i])

    def qkv_copy(m, q):
        cols = pl.ds(256 * q, 256)
        return pltpu.make_async_copy(wqkv[m][0].at[:, cols], wqkv[m][1].at[:, cols], sem_q.at[m, q])

    def x_copy(i):
        return pltpu.make_async_copy(x_hbm.at[pl.ds(i * L, L)], xio.at[pl.ds(i * L, L)], sem_x.at[i])

    def o_copy(i):
        r = pl.multiple_of(i * BM, BM)
        return pltpu.make_async_copy(xio.at[pl.ds(r, BM)], out_hbm.at[pl.ds(r, BM)], sem_o.at[i])

    x_copy(0).start()
    qkv_copy(0, 0).start()
    qkv_copy(1, 0).start()
    x_copy(1).start()
    qkv_copy(2, 0).start()

    gt[...] = jax.nn.sigmoid(beta_ref[...])
    hb[0:8, :] = jnp.zeros((8, D), f32)
    hb[8 + S_LEN:16 + S_LEN, :] = jnp.zeros((8, D), f32)
    pb[...] = jnp.zeros(pb.shape, i32)
    rb[...] = jnp.zeros(rb.shape, f32)
    vt[...] = jnp.zeros(vt.shape, i32)
    pk[3] = jnp.zeros(pk.shape[1:], i32)

    def unit(u):
        return u // G, u % G

    def xs_of(s):
        return i2b(xn[pl.ds(pl.multiple_of(s * (L // 2), L // 2), L // 2), :])

    def col(g):
        return pl.ds(pl.multiple_of(g * 128, 128), 128)

    def rows64(c):
        return pl.ds(pl.multiple_of(c * 64, 64), 64), pl.ds(pl.multiple_of(c * 32, 32), 32)

    def rowsn(c, n):
        return pl.ds(pl.multiple_of(c * n, n), n), pl.ds(pl.multiple_of(c * (n // 2), n // 2), n // 2)

    def XN(c, rep, n=64):
        r, rp = rowsn(c, n)
        x = jnp.where(rep == 0, xio[r, :].astype(f32), xf[r, :])
        xf[r, :] = x
        xn[rp, :] = b2i(_ln(x).astype(bf16))

    def LNLN(c, n=64):
        r, rp = rowsn(c, n)
        z, y = _ln2(xf[r, :])
        zf[r, :] = z
        y1[rp, :] = b2i(y.astype(bf16))

    def D1q(u):
        s, g = unit(u)
        q = _dot(xs_of(s), wq[:, col(g)])
        qs[...] = b2i((q * QSCALE).astype(bf16))
        pq[u % 4] = b2i(_phi(q).astype(bf16))

    def D1k(u):
        s, g = unit(u)
        k = _dot(xs_of(s), wk[:, col(g)])
        kb[...] = b2i(k.astype(bf16))
        pk[u % 4] = b2i(_phi(k).astype(bf16))

    def D1v(u):
        s, g = unit(u)
        v = _dot(xs_of(s), wv[:, col(g)])
        vt[...] = b2i(v.astype(bf16).T)

    def S_stage(j):
        n = 128 * (j + 1)
        lane = lax.broadcasted_iota(i32, (64, 128), 1)
        hm = [jnp.where((lane >= 32 * h) & (lane < 32 * h + 32), -1, 0).astype(i32) for h in range(4)]
        valid = lax.broadcasted_iota(i32, (128, 128), 0) <= lax.broadcasted_iota(i32, (128, 128), 1)
        k4 = i2b(kb[:n // 2, :])
        qj = qs[64 * j:64 * j + 64, :]
        qst = i2b(jnp.concatenate([qj & hm[h] for h in range(4)], axis=0))
        sT = lax.dot_general(k4, qst, NT, preferred_element_type=f32)
        for h in range(4):
            sh = sT[:, 128 * h:128 * h + 128]
            dg = jnp.where(valid, sh[128 * j:], NEG)
            sh = jnp.concatenate([sh[:128 * j], dg], axis=0) if j else dg
            sb[OFF[j]:OFF[j] + n, 128 * h:128 * h + 128] = sh
            m = jnp.max(sh, axis=0, keepdims=True)
            mb[8 * j:8 * j + 8, 128 * h:128 * h + 128] = jnp.broadcast_to(m, (8, 128))

    def E_stage(j):
        for h in range(4):
            m = mb[8 * j:8 * j + 8, 128 * h:128 * h + 128]
            l = None
            for i in range(j + 1):
                r0 = OFF[j] + 128 * i
                s = sb[r0:r0 + 128, 128 * h:128 * h + 128]
                p = jnp.exp2(s.reshape(16, 8, 128) - m[None])
                li = jnp.sum(p, axis=0)
                l = li if l is None else l + li
                pb[r0 // 2:r0 // 2 + 64, 128 * h:128 * h + 128] = b2i(p.reshape(128, 128).astype(bf16))
            lt = jnp.sum(l, axis=0, keepdims=True)
            rb[8 * j:8 * j + 8, 128 * h:128 * h + 128] = jnp.broadcast_to(1.0 / lt, (8, 128))

    def gate8(g, h):
        return gt[pl.ds(pl.multiple_of(g * 32 + 8 * h, 8), 8), :]

    def V_dots(j, u):
        s, g = unit(u)
        n = 128 * (j + 1)
        outs = []
        for h in range(4):
            vh = i2b(vt[16 * h:16 * h + 16, :n])
            p = i2b(pb[OFF[j] // 2:(OFF[j] + n) // 2, 128 * h:128 * h + 128])
            oT = _dot(vh, p)
            r = rb[8 * j:8 * j + 8, 128 * h:128 * h + 128] * (1.0 - gate8(g, h))
            outs.append((oT.reshape(4, 8, 128) * r[None]).reshape(32, 128))
        return jnp.concatenate(outs, axis=0)

    def M_read(u):
        s, g = unit(u)
        mtb = mt[g].astype(bf16)
        nd = lax.dot_general(mtb, i2b(pq[u % 4]), NT, preferred_element_type=f32)
        outs = []
        for h in range(4):
            den = jnp.broadcast_to(nd[128 + h:129 + h], (8, 512)) + 1e-6
            c = jnp.concatenate([gate8(g, h)] * 4, axis=1) / den
            outs.append((nd[32 * h:32 * h + 32].reshape(4, 8, 512) * c[None]).reshape(32, 512))
        return jnp.concatenate(outs, axis=0)

    def V_finish(u, adots, amem):
        s, g = unit(u)
        o = jnp.concatenate(adots, axis=1)
        if amem is not None:
            o = o + amem
        ob[pl.ds(pl.multiple_of(s * 256, 256), 256), col(g)] = b2i(o.astype(bf16).T)

    def M_update(u, first_seg):
        s, g = unit(u)
        ones = jnp.full((8, 512), 0x3F803F80, i32)
        lhs = i2b(jnp.concatenate([vt[...], ones], axis=0))
        upd = _dot(lhs, i2b(pk[u % 4]))
        r = lax.broadcasted_iota(i32, (144, 128), 0)
        c = lax.broadcasted_iota(i32, (144, 128), 1)
        rh = jnp.where(r < 128, r // 32, r - 128)
        upd = jnp.where(rh == c // 32, upd, 0.0)
        if first_seg:
            mt[g] = upd
        else:
            mt[g] = mt[g] + upd

    def D2(v):
        s, c = unit(v)
        o = i2b(ob[pl.ds(pl.multiple_of(s * 256, 256), 256), :])
        y = _dot(o, wo[:, col(c)])
        rows = pl.ds(pl.multiple_of(s * L, L), L)
        xf[rows, col(c)] = xf[rows, col(c)] + y

    def a_iter(t, rep, on, first_seg=False, order="order1"):
        adots = [None] * 4
        amem = None
        uv = jnp.maximum(t - 1, 0)
        for tok in cfg[order].split():
            k = tok[0]
            if k not in on:
                continue
            if k == "V":
                adots[int(tok[1])] = V_dots(int(tok[1]), uv)
            elif k == "E":
                E_stage(int(tok[1]))
            elif k == "S":
                S_stage(int(tok[1]))
            elif k == "D":
                D2(t - 9)
            elif k == "X":
                XN(jnp.minimum(t + 10, 31), rep)
            elif k == "N":
                LNLN(jnp.maximum(t - 17, 0))
            elif k == "R":
                if not first_seg:
                    amem = M_read(uv)
            elif k == "F":
                V_finish(uv, adots, amem)
            elif k == "U":
                M_update(uv, first_seg)
            elif k == "Q":
                D1q(jnp.minimum(t + 2, NU - 1))
            elif k == "K":
                D1k(jnp.minimum(t + 2, NU - 1))
            elif k == "W":
                D1v(t)

    def ba_body(i, c):
        lhs = i2b(y1[pl.ds(pl.multiple_of(i * (BM // 2), BM // 2), BM // 2), :])
        hb[pl.ds(pl.multiple_of(i * BM + 8, 8), BM), :] = _gelu(_dot(lhs, w1[...]))
        return c

    def shifted(r0):
        win_ = hb[pl.ds(pl.multiple_of(r0, 8), 144), :]
        parts = []
        for gi, sh in enumerate((-1, 1, -2, 2)):
            parts.append(win_[8 + sh:8 + sh + 128, 256 * gi:256 * gi + 256])
        return jnp.concatenate(parts, axis=1).astype(bf16)

    def bb_body(i, rep):
        rows = [pl.multiple_of(i * BM + 128 * a, 128) for a in range(2)]
        x1 = [zf[pl.ds(r, 128), :] + _dot(shifted(r), w2[...]) for r in rows]
        y2 = [_ln(v).astype(bf16) for v in x1]
        gg = [_gelu(_dot(y2[a], w3[...])).astype(bf16) for a in range(2)]
        for a in range(2):
            r = rows[a]
            xo = xf[pl.ds(r, 128), :] + x1[a] + _dot(gg[a], w4[...])
            xf[pl.ds(r, 128), :] = xo
            xio[pl.ds(r, 128), :] = xo.astype(bf16)

        @pl.when(rep == 1)
        def _():
            o_copy(i).start()
        return rep

    ALL = "VESDXNRFUQKW"

    def l1(t, rep):
        for tt, wi in ((2, 0), (4, 1), (6, 2)):
            @pl.when((rep == 0) & (t == tt))
            def _():
                w_copy(wi).start()
        for tt, q in ((2, 2), (4, 3)):
            @pl.when((rep == 0) & (t == tt))
            def _():
                for m in range(3):
                    qkv_copy(m, q).wait()

        @pl.when((rep == 0) & (t == 6))
        def _():
            x_copy(2).wait()
        a_iter(t, rep, "VESXRFUQKW", first_seg=True)
        return rep

    def l2(t, rep):
        for tt, wi in ((11, 3), (16, 4)):
            @pl.when((rep == 0) & (t == tt))
            def _():
                w_copy(wi).start()

        @pl.when((rep == 0) & (t == 14))
        def _():
            x_copy(3).wait()
        a_iter(t, rep, ALL, order="order2")
        return rep

    if cfg["mode"] == "l2":
        lax.fori_loop(9, 30, l2, 0)
        return
    if cfg["mode"] == "l1":
        lax.fori_loop(0, 9, l1, 0)
        return
    if cfg["mode"] == "bb":
        lax.fori_loop(0, NB, bb_body, 0)
        return

    def rep_body(rep, c):
        with scope("z_xn0"):
            @pl.when(rep == 0)
            def _():
                x_copy(0).wait()

            def xn0(c_, carry):
                XN(c_, rep, 128)
                return carry
            lax.fori_loop(0, 4, xn0, 0)

        with scope("z_apro"):
            @pl.when(rep == 0)
            def _():
                qkv_copy(0, 0).wait()
                qkv_copy(1, 0).wait()
            a_iter(-2, rep, "QK")

            @pl.when(rep == 0)
            def _():
                x_copy(1).wait()
                qkv_copy(2, 0).wait()
                for m in range(3):
                    qkv_copy(m, 1).start()
            XN(8, rep)
            XN(9, rep)
            a_iter(-1, rep, "SQK")

            @pl.when(rep == 0)
            def _():
                for m in range(3):
                    qkv_copy(m, 1).wait()
                for q in (2, 3):
                    for m in range(3):
                        qkv_copy(m, q).start()
                x_copy(2).start()
                x_copy(3).start()

        with scope("z_l1"):
            lax.fori_loop(0, 9, l1, rep)

        @pl.when(rep == 0)
        def _():
            w_copy(0).wait()

        with scope("z_l2"):
            lax.fori_loop(9, 30, l2, rep)
        with scope("z_aepi"):
            a_iter(30, rep, "VESDNRFW", order="order3")
            a_iter(31, rep, "VEDNRFW", order="order3")
            a_iter(32, rep, "VDNRF", order="order3")

        def l3(t, c):
            a_iter(t, rep, "DN", order="order3")
            return c
        with scope("z_l3"):
            lax.fori_loop(33, 41, l3, 0)

        @pl.when(rep == 0)
        def _():
            for i in range(1, 5):
                w_copy(i).wait()

        def ln3(c_, carry):
            LNLN(c_, 128)
            return carry
        with scope("z_ln3"):
            lax.fori_loop(12, 16, ln3, 0)
        if cfg["mode"] != "A":
            with scope("z_ba"):
                lax.fori_loop(0, NB, ba_body, 0)
            with scope("z_bb"):
                lax.fori_loop(0, NB, bb_body, rep)
        return c

    lax.fori_loop(0, 2, rep_body, 0)
    with scope("z_owait"):
        for i in range(NB):
            o_copy(i).wait()


def build(cfg, name="infini_mixer"):
    vm = pltpu.VMEM
    scratch = [
        vm((S_LEN, D), bf16),
        vm((D, D), bf16), vm((D, D), bf16), vm((D, D), bf16), vm((D, D), bf16),
        vm((D, D), bf16), vm((D, D), bf16), vm((D, F), bf16), vm((F, D), bf16),
        vm((S_LEN, D), f32),
        vm((S_LEN, D), f32),
        vm((S_LEN // 2, D), i32),
        vm((S_LEN // 2, D), i32),
        vm((256, 128), i32), vm((256, 128), i32),
        vm((4, 256, 128), i32), vm((4, 256, 128), i32),
        vm((64, 512), i32),
        vm((1280, 512), f32), vm((640, 512), i32),
        vm((32, 512), f32), vm((32, 512), f32),
        vm((S_LEN // 2, D), i32),
        vm((G, 144, 128), f32),
        vm((S_LEN + 16, D), f32),
        vm((H * 8, 128), f32),
        pltpu.SemaphoreType.DMA((4,)), pltpu.SemaphoreType.DMA((3, 4)),
        pltpu.SemaphoreType.DMA((5,)), pltpu.SemaphoreType.DMA((NB,)),
    ]
    any_spec = pl.BlockSpec(memory_space=pl.ANY)
    return pl.pallas_call(
        functools.partial(_kernel, cfg=cfg),
        out_shape=jax.ShapeDtypeStruct((S_LEN, D), bf16),
        in_specs=[any_spec] * 5 + [pl.BlockSpec(memory_space=pltpu.VMEM)] + [any_spec] * 4,
        out_specs=any_spec,
        scratch_shapes=scratch,
        compiler_params=pltpu.CompilerParams(vmem_limit_bytes=110 * 2 ** 20),
        name=name,
    )


def make_kernel(cfg, name="infini_mixer"):
    def pallas_interleave_layers__memory_aug_infini_attn__mixer_s_mlp__prompt_kernel(A_x, A_wq, A_wk, A_wv, A_wo, A_beta, B_x, B_w1, B_w2, B_w3, B_w4):
        beta = jnp.broadcast_to(A_beta.astype(f32).reshape(H, 1, 1), (H, 8, 128)).reshape(H * 8, 128)
        out = build(cfg, name)(A_x.reshape(S_LEN, D), A_wq, A_wk, A_wv, A_wo, beta, B_w1, B_w2, B_w3, B_w4)
        return out.reshape(1, S_LEN, D)
    return jax.jit(kernel)


kernel = make_kernel(CFG)
```

```python
import functools
import math

import numpy as np
import jax
import jax.numpy as jnp
from jax import lax
import jax.experimental.pallas as pl
import jax.experimental.pallas.tpu as pltpu

S_LEN = 2048
D = 1024
F = 3584
H = 32
DH = 32
NSEG = 4
L = 512
G = 8
NU = NSEG * G
OFF = (0, 128, 384, 768)
EPS = 1e-5
QSCALE = float(DH ** -0.5 * math.log2(math.e))
NEG = -1e30
BM = 256
NB = S_LEN // BM

f32 = jnp.float32
bf16 = jnp.bfloat16
i32 = jnp.int32
NT = (((1,), (1,)), ((), ()))

CONSTRAINTS = [("E.", "V#"), ("E.", "S#"), ("V.", "W"), ("U", "W"), ("S.", "Q"), ("S.", "K"), ("R", "U"), ("V.", "F"), ("R", "F")]
SEARCH_MODE = "A"
SEARCH_T = 400.0


def score(loops, total):
    rep, xn0, l1, l2, l3, ln3 = loops[:6]
    ln = lambda x: x[1] - x[0]
    straight = ln(rep) - ln(xn0) - ln(l1) - ln(l2) - ln(l3) - ln(ln3)
    parts = [ln(xn0), ln(l1), ln(l2), ln(l3), ln(ln3), straight]
    return 4 * ln(xn0) + 8 * ln(l1) + 22 * ln(l2) + 8 * ln(l3) + 4 * ln(ln3) + straight, parts


COMPONENTS = {"order1": (lambda p: p[1], 25.0), "order2": (lambda p: p[2], 25.0), "order3": (lambda p: 8 * p[3] + p[5], 50.0)}
CFG = dict(
    order1="E1 E0 E2 S0 S2 E3 V2 N S1 S3 K V3 V0 V1 R U W Q D X F",
    order2="E0 E3 S3 E1 V0 S0 S1 E2 V1 X S2 R D K N V2 V3 U W F Q",
    order3="N E1 E0 E2 S1 V1 E3 S0 S3 V3 S2 V2 R V0 U Q F K W D X",
    mode="full",
    scopes=False,
)


def i2b(x):
    return pltpu.bitcast(x, bf16)


def b2i(x):
    return pltpu.bitcast(x, i32)


def _ln(x):
    m = jnp.mean(x, axis=-1, keepdims=True)
    d = x - m
    v = jnp.mean(d * d, axis=-1, keepdims=True)
    return d * lax.rsqrt(v + EPS)


def _ln2(x):
    m = jnp.mean(x, axis=-1, keepdims=True)
    d = x - m
    v = jnp.mean(d * d, axis=-1, keepdims=True)
    r = lax.rsqrt(v + EPS)
    r2 = r * lax.rsqrt(v * r * r + EPS)
    return d * r, d * r2


def _gelu(x):
    c0 = math.sqrt(2.0 / math.pi)
    c1 = c0 * 0.044715
    return (0.5 * x) * (1.0 + jnp.tanh(x * (c0 + c1 * (x * x))))


def _phi(t):
    return jnp.where(t > 0, t + 1.0, jnp.exp(t))


def _dot(a, b):
    return jnp.dot(a, b, preferred_element_type=f32)


class _NoScope:
    def __enter__(self):
        return self

    def __exit__(self, *a):
        return False


def _kernel(x_hbm, wq_hbm, wk_hbm, wv_hbm, wo_hbm, beta_ref, w1_hbm, w2_hbm, w3_hbm, w4_hbm,
            out_hbm,
            xio, wq, wk, wv, wo, w1, w2, w3, w4,
            xf, zf, xn, y1, qs, kb, pq, pk, vt, sb, mb, ob, mt, hb, gt,
            sem_x, sem_q, sem_w, sem_o, *, cfg):
    scope = jax.named_scope if cfg["scopes"] else (lambda name: _NoScope())
    wlate = [(wo_hbm, wo), (w1_hbm, w1), (w2_hbm, w2), (w3_hbm, w3), (w4_hbm, w4)]
    wqkv = [(wq_hbm, wq), (wk_hbm, wk), (wv_hbm, wv)]

    def w_copy(i):
        return pltpu.make_async_copy(wlate[i][0], wlate[i][1], sem_w.at[i])

    def qkv_copy(m, q):
        cols = pl.ds(256 * q, 256)
        return pltpu.make_async_copy(wqkv[m][0].at[:, cols], wqkv[m][1].at[:, cols], sem_q.at[m, q])

    def x_copy(i):
        return pltpu.make_async_copy(x_hbm.at[pl.ds(i * L, L)], xio.at[pl.ds(i * L, L)], sem_x.at[i])

    def o_copy(i):
        r = pl.multiple_of(i * BM, BM)
        return pltpu.make_async_copy(xio.at[pl.ds(r, BM)], out_hbm.at[pl.ds(r, BM)], sem_o.at[i])

    x_copy(0).start()
    qkv_copy(0, 0).start()
    qkv_copy(1, 0).start()
    x_copy(1).start()
    qkv_copy(2, 0).start()

    gt[...] = jax.nn.sigmoid(beta_ref[...])
    hb[0:8, :] = jnp.zeros((8, D), f32)
    hb[8 + S_LEN:16 + S_LEN, :] = jnp.zeros((8, D), f32)

    def unit(u):
        return u // G, u % G

    def xs_of(s):
        return i2b(xn[pl.ds(pl.multiple_of(s * (L // 2), L // 2), L // 2), :])

    def col(g):
        return pl.ds(pl.multiple_of(g * 128, 128), 128)

    def rows64(c):
        return pl.ds(pl.multiple_of(c * 64, 64), 64), pl.ds(pl.multiple_of(c * 32, 32), 32)

    def rowsn(c, n):
        return pl.ds(pl.multiple_of(c * n, n), n), pl.ds(pl.multiple_of(c * (n // 2), n // 2), n // 2)

    def XN(c, rep, n=64):
        r, rp = rowsn(c, n)
        x = jnp.where(rep == 0, xio[r, :].astype(f32), xf[r, :])
        xf[r, :] = x
        xn[rp, :] = b2i(_ln(x).astype(bf16))

    def LNLN(c, n=64):
        r, rp = rowsn(c, n)
        z, y = _ln2(xf[r, :])
        zf[r, :] = z
        y1[rp, :] = b2i(y.astype(bf16))

    def D1q(u):
        s, g = unit(u)
        q = _dot(xs_of(s), wq[:, col(g)])
        qs[...] = b2i((q * QSCALE).astype(bf16))
        pq[u % 4] = b2i(_phi(q).astype(bf16))

    def D1k(u):
        s, g = unit(u)
        k = _dot(xs_of(s), wk[:, col(g)])
        kb[...] = b2i(k.astype(bf16))
        pk[u % 4] = b2i(_phi(k).astype(bf16))

    def D1v(u):
        s, g = unit(u)
        v = _dot(xs_of(s), wv[:, col(g)])
        vt[...] = b2i(v.astype(bf16).T)

    def S_stage(j):
        n = 128 * (j + 1)
        lane = lax.broadcasted_iota(i32, (64, 128), 1)
        hm = [jnp.where((lane >= 32 * h) & (lane < 32 * h + 32), -1, 0).astype(i32) for h in range(4)]
        valid = lax.broadcasted_iota(i32, (128, 128), 0) <= lax.broadcasted_iota(i32, (128, 128), 1)
        k4 = i2b(kb[:n // 2, :])
        qj = qs[64 * j:64 * j + 64, :]
        qst = i2b(jnp.concatenate([qj & hm[h] for h in range(4)], axis=0))
        sT = lax.dot_general(k4, qst, NT, preferred_element_type=f32)
        for h in range(4):
            sh = sT[:, 128 * h:128 * h + 128]
            dg = jnp.where(valid, sh[128 * j:], NEG)
            sh = jnp.concatenate([sh[:128 * j], dg], axis=0) if j else dg
            sb[OFF[j]:OFF[j] + n, 128 * h:128 * h + 128] = sh
            m = jnp.max(sh, axis=0, keepdims=True)
            mb[8 * j:8 * j + 8, 128 * h:128 * h + 128] = jnp.broadcast_to(m, (8, 128))

    def E_stage(j, u):
        s_, g = unit(u)
        ps, rs = [], []
        for h in range(4):
            m = mb[8 * j:8 * j + 8, 128 * h:128 * h + 128]
            l = None
            pt = []
            for i in range(j + 1):
                r0 = OFF[j] + 128 * i
                s = sb[r0:r0 + 128, 128 * h:128 * h + 128]
                p = jnp.exp2(s.reshape(16, 8, 128) - m[None])
                li = jnp.sum(p, axis=0)
                l = li if l is None else l + li
                pt.append(p.reshape(128, 128).astype(bf16))
            lt = jnp.sum(l, axis=0, keepdims=True)
            rs.append(jnp.broadcast_to(1.0 / lt, (8, 128)) * (1.0 - gate8(g, h)))
            ps.append(pt)
        return ps, rs

    def gate8(g, h):
        return gt[pl.ds(pl.multiple_of(g * 32 + 8 * h, 8), 8), :]

    def V_dots(j, ps, rs):
        outs = []
        for h in range(4):
            acc = None
            for i in range(j + 1):
                vh = i2b(vt[16 * h:16 * h + 16, 128 * i:128 * i + 128])
                d = _dot(vh, ps[h][i])
                acc = d if acc is None else acc + d
            outs.append((acc.reshape(4, 8, 128) * rs[h][None]).reshape(32, 128))
        return jnp.concatenate(outs, axis=0)

    def M_read(u):
        s, g = unit(u)
        mtb = mt[g].astype(bf16)
        nd = lax.dot_general(mtb, i2b(pq[u % 4]), NT, preferred_element_type=f32)
        outs = []
        for h in range(4):
            den = jnp.broadcast_to(nd[128 + h:129 + h], (8, 512)) + 1e-6
            c = jnp.concatenate([gate8(g, h)] * 4, axis=1) / den
            outs.append((nd[32 * h:32 * h + 32].reshape(4, 8, 512) * c[None]).reshape(32, 512))
        return jnp.concatenate(outs, axis=0)

    def V_finish(u, adots, amem):
        s, g = unit(u)
        o = jnp.concatenate(adots, axis=1)
        if amem is not None:
            o = o + amem
        ob[pl.ds(pl.multiple_of(s * 256, 256), 256), col(g)] = b2i(o.astype(bf16).T)

    def M_update(u, first_seg):
        s, g = unit(u)
        ones = jnp.full((8, 512), 0x3F803F80, i32)
        lhs = i2b(jnp.concatenate([vt[...], ones], axis=0))
        upd = _dot(lhs, i2b(pk[u % 4]))
        r = lax.broadcasted_iota(i32, (144, 128), 0)
        c = lax.broadcasted_iota(i32, (144, 128), 1)
        rh = jnp.where(r < 128, r // 32, r - 128)
        upd = jnp.where(rh == c // 32, upd, 0.0)
        if first_seg:
            mt[g] = upd
        else:
            mt[g] = mt[g] + upd

    def D2(v):
        s, c = unit(v)
        o = i2b(ob[pl.ds(pl.multiple_of(s * 256, 256), 256), :])
        y = _dot(o, wo[:, col(c)])
        rows = pl.ds(pl.multiple_of(s * L, L), L)
        xf[rows, col(c)] = xf[rows, col(c)] + y

    def a_iter(t, rep, on, first_seg=False, order="order1"):
        adots = [None] * 4
        pr = [None] * 4
        amem = None
        for tok in cfg[order].split():
            k = tok[0]
            if k not in on:
                continue
            if k == "V":
                adots[int(tok[1])] = V_dots(int(tok[1]), *pr[int(tok[1])])
            elif k == "E":
                pr[int(tok[1])] = E_stage(int(tok[1]), t)
            elif k == "S":
                S_stage(int(tok[1]))
            elif k == "D":
                D2(t - 8)
            elif k == "X":
                XN(jnp.minimum(t + 10, 31), rep)
            elif k == "N":
                LNLN(jnp.maximum(t - 16, 0))
            elif k == "R":
                if not first_seg:
                    amem = M_read(t)
            elif k == "F":
                V_finish(t, adots, amem)
            elif k == "U":
                M_update(t, first_seg)
            elif k == "Q":
                D1q(t + 2)
            elif k == "K":
                D1k(t + 2)
            elif k == "W":
                D1v(t + 1)

    def ba_body(i, c):
        lhs = i2b(y1[pl.ds(pl.multiple_of(i * (BM // 2), BM // 2), BM // 2), :])
        hb[pl.ds(pl.multiple_of(i * BM + 8, 8), BM), :] = _gelu(_dot(lhs, w1[...]))
        return c

    def shifted(r0):
        win_ = hb[pl.ds(pl.multiple_of(r0, 8), 144), :]
        parts = []
        for gi, sh in enumerate((-1, 1, -2, 2)):
            parts.append(win_[8 + sh:8 + sh + 128, 256 * gi:256 * gi + 256])
        return jnp.concatenate(parts, axis=1).astype(bf16)

    def bb_body(i, rep):
        rows = [pl.multiple_of(i * BM + 128 * a, 128) for a in range(2)]
        x1 = [zf[pl.ds(r, 128), :] + _dot(shifted(r), w2[...]) for r in rows]
        y2 = [_ln(v).astype(bf16) for v in x1]
        gg = [_gelu(_dot(y2[a], w3[...])).astype(bf16) for a in range(2)]
        for a in range(2):
            r = rows[a]
            xo = xf[pl.ds(r, 128), :] + x1[a] + _dot(gg[a], w4[...])
            xf[pl.ds(r, 128), :] = xo
            xio[pl.ds(r, 128), :] = xo.astype(bf16)

        @pl.when(rep == 1)
        def _():
            o_copy(i).start()
        return rep

    ALL = "VESDXNRFUQKW"

    def l1(t, rep):
        for tt, wi in ((2, 0), (4, 1), (6, 2)):
            @pl.when((rep == 0) & (t == tt))
            def _():
                w_copy(wi).start()
        for tt, q in ((2, 2), (4, 3)):
            @pl.when((rep == 0) & (t == tt))
            def _():
                for m in range(3):
                    qkv_copy(m, q).wait()

        @pl.when((rep == 0) & (t == 6))
        def _():
            x_copy(2).wait()
        a_iter(t, rep, "VESXRFUQKW", first_seg=True)
        return rep

    def l2(t, rep):
        for tt, wi in ((11, 3), (16, 4)):
            @pl.when((rep == 0) & (t == tt))
            def _():
                w_copy(wi).start()

        @pl.when((rep == 0) & (t == 14))
        def _():
            x_copy(3).wait()
        a_iter(t, rep, ALL, order="order2")
        return rep

    if cfg["mode"] == "l2":
        lax.fori_loop(8, 30, l2, 0)
        return
    if cfg["mode"] == "l1":
        lax.fori_loop(0, 8, l1, 0)
        return
    if cfg["mode"] == "bb":
        lax.fori_loop(0, NB, bb_body, 0)
        return

    def rep_body(rep, c):
        with scope("z_xn0"):
            @pl.when(rep == 0)
            def _():
                x_copy(0).wait()

            def xn0(c_, carry):
                XN(c_, rep, 128)
                return carry
            lax.fori_loop(0, 4, xn0, 0)

        with scope("z_apro"):
            @pl.when(rep == 0)
            def _():
                qkv_copy(0, 0).wait()
                qkv_copy(1, 0).wait()
            a_iter(-2, rep, "QK")

            @pl.when(rep == 0)
            def _():
                x_copy(1).wait()
                qkv_copy(2, 0).wait()
                for m in range(3):
                    qkv_copy(m, 1).start()
            XN(8, rep)
            XN(9, rep)
            a_iter(-1, rep, "SWQK")

            @pl.when(rep == 0)
            def _():
                for m in range(3):
                    qkv_copy(m, 1).wait()
                for q in (2, 3):
                    for m in range(3):
                        qkv_copy(m, q).start()
                x_copy(2).start()
                x_copy(3).start()

        with scope("z_l1"):
            lax.fori_loop(0, 8, l1, rep)

        @pl.when(rep == 0)
        def _():
            w_copy(0).wait()

        with scope("z_l2"):
            lax.fori_loop(8, 30, l2, rep)
        with scope("z_aepi"):
            a_iter(30, rep, "VESDNRFW", order="order3")
            a_iter(31, rep, "VEDNRF", order="order3")

        def l3(t, c):
            a_iter(t, rep, "DN", order="order3")
            return c
        with scope("z_l3"):
            lax.fori_loop(32, 40, l3, 0)

        @pl.when(rep == 0)
        def _():
            for i in range(1, 5):
                w_copy(i).wait()

        def ln3(c_, carry):
            LNLN(c_, 128)
            return carry
        with scope("z_ln3"):
            lax.fori_loop(12, 16, ln3, 0)
        if cfg["mode"] != "A":
            with scope("z_ba"):
                lax.fori_loop(0, NB, ba_body, 0)
            with scope("z_bb"):
                lax.fori_loop(0, NB, bb_body, rep)
        return c

    lax.fori_loop(0, 2, rep_body, 0)
    with scope("z_owait"):
        for i in range(NB):
            o_copy(i).wait()


def build(cfg, name="infini_mixer"):
    vm = pltpu.VMEM
    scratch = [
        vm((S_LEN, D), bf16),
        vm((D, D), bf16), vm((D, D), bf16), vm((D, D), bf16), vm((D, D), bf16),
        vm((D, D), bf16), vm((D, D), bf16), vm((D, F), bf16), vm((F, D), bf16),
        vm((S_LEN, D), f32),
        vm((S_LEN, D), f32),
        vm((S_LEN // 2, D), i32),
        vm((S_LEN // 2, D), i32),
        vm((256, 128), i32), vm((256, 128), i32),
        vm((4, 256, 128), i32), vm((4, 256, 128), i32),
        vm((64, 512), i32),
        vm((1280, 512), f32), vm((32, 512), f32),
        vm((S_LEN // 2, D), i32),
        vm((G, 144, 128), f32),
        vm((S_LEN + 16, D), f32),
        vm((H * 8, 128), f32),
        pltpu.SemaphoreType.DMA((4,)), pltpu.SemaphoreType.DMA((3, 4)),
        pltpu.SemaphoreType.DMA((5,)), pltpu.SemaphoreType.DMA((NB,)),
    ]
    any_spec = pl.BlockSpec(memory_space=pl.ANY)
    return pl.pallas_call(
        functools.partial(_kernel, cfg=cfg),
        out_shape=jax.ShapeDtypeStruct((S_LEN, D), bf16),
        in_specs=[any_spec] * 5 + [pl.BlockSpec(memory_space=pltpu.VMEM)] + [any_spec] * 4,
        out_specs=any_spec,
        scratch_shapes=scratch,
        compiler_params=pltpu.CompilerParams(vmem_limit_bytes=110 * 2 ** 20),
        name=name,
    )


def make_kernel(cfg, name="infini_mixer"):
    def pallas_interleave_layers__memory_aug_infini_attn__mixer_s_mlp__prompt_kernel(A_x, A_wq, A_wk, A_wv, A_wo, A_beta, B_x, B_w1, B_w2, B_w3, B_w4):
        beta = jnp.broadcast_to(A_beta.astype(f32).reshape(H, 1, 1), (H, 8, 128)).reshape(H * 8, 128)
        out = build(cfg, name)(A_x.reshape(S_LEN, D), A_wq, A_wk, A_wv, A_wo, beta, B_w1, B_w2, B_w3, B_w4)
        return out.reshape(1, S_LEN, D)
    return jax.jit(kernel)


kernel = make_kernel(CFG)
```

```python
import functools
import math

import numpy as np
import jax
import jax.numpy as jnp
from jax import lax
import jax.experimental.pallas as pl
import jax.experimental.pallas.tpu as pltpu

S_LEN = 2048
D = 1024
F = 3584
H = 32
DH = 32
NSEG = 4
L = 512
G = 8
NU = NSEG * G
OFF = (0, 128, 384, 768)
EPS = 1e-5
QSCALE = float(DH ** -0.5 * math.log2(math.e))
NEG = -1e30
BM = 256
NB = S_LEN // BM

f32 = jnp.float32
bf16 = jnp.bfloat16
i32 = jnp.int32
NT = (((1,), (1,)), ((), ()))

CONSTRAINTS = [("E.", "V#"), ("E.", "S#"), ("V.", "W"), ("U", "W"), ("S.", "Q"), ("S.", "K"), ("R", "U"), ("V.", "F"), ("R", "F")]
SEARCH_MODE = "A"
SEARCH_T = 400.0


def score(loops, total):
    rep, xn0, l1, l2, t1, t2 = loops[:6]
    ln = lambda x: x[1] - x[0]
    straight = ln(rep) - ln(xn0) - ln(l1) - ln(l2) - ln(t1) - ln(t2)
    parts = [ln(xn0), ln(l1), ln(l2), ln(t1), ln(t2), straight]
    return 4 * ln(xn0) + 8 * ln(l1) + 22 * ln(l2) + 4 * ln(t1) + 4 * ln(t2) + straight, parts


COMPONENTS = {"order1": (lambda p: p[1], 25.0), "order2": (lambda p: p[2], 25.0), "order3": (lambda p: p[5], 30.0),
              "order4": (lambda p: p[3], 30.0), "order5": (lambda p: p[4], 30.0)}
CFG = dict(
    order1="E1 E0 E2 S0 S2 E3 V2 N S1 S3 K V3 V0 V1 R U W Q D X F",
    order2="E0 E3 S3 E1 V0 S0 S1 E2 V1 X S2 R D K N V2 V3 U W F Q",
    order3="N E1 E0 E2 S1 V1 E3 S0 S3 V3 S2 V2 R V0 U Q F K W D X",
    order4="N D0 B0 D1 B1",
    order5="B0 N0 B1 N1",
    mode="full",
    scopes=False,
)


def i2b(x):
    return pltpu.bitcast(x, bf16)


def b2i(x):
    return pltpu.bitcast(x, i32)


def _ln(x):
    m = jnp.mean(x, axis=-1, keepdims=True)
    d = x - m
    v = jnp.mean(d * d, axis=-1, keepdims=True)
    return d * lax.rsqrt(v + EPS)


def _ln2(x):
    m = jnp.mean(x, axis=-1, keepdims=True)
    d = x - m
    v = jnp.mean(d * d, axis=-1, keepdims=True)
    r = lax.rsqrt(v + EPS)
    r2 = r * lax.rsqrt(v * r * r + EPS)
    return d * r, d * r2


def _gelu(x):
    c0 = math.sqrt(2.0 / math.pi)
    c1 = c0 * 0.044715
    return (0.5 * x) * (1.0 + jnp.tanh(x * (c0 + c1 * (x * x))))


def _phi(t):
    return jnp.where(t > 0, t + 1.0, jnp.exp(t))


def _dot(a, b):
    return jnp.dot(a, b, preferred_element_type=f32)


class _NoScope:
    def __enter__(self):
        return self

    def __exit__(self, *a):
        return False


def _kernel(x_hbm, wq_hbm, wk_hbm, wv_hbm, wo_hbm, beta_hbm, w1_hbm, w2_hbm, w3_hbm, w4_hbm,
            out_hbm,
            xio, wq, wk, wv, wo, w1, w2, w3, w4,
            xf, zf, xn, y1, qs, kb, pq, pk, vt, sb, mb, ob, mt, hb, gt, bt,
            sem_x, sem_q, sem_w, sem_o, sem_b, sem_x0, *, cfg):
    scope = jax.named_scope if cfg["scopes"] else (lambda name: _NoScope())
    wlate = [(wo_hbm, wo), (w1_hbm, w1), (w2_hbm, w2), (w3_hbm, w3), (w4_hbm, w4)]
    wqkv = [(wq_hbm, wq), (wk_hbm, wk), (wv_hbm, wv)]

    def w_copy(i):
        return pltpu.make_async_copy(wlate[i][0], wlate[i][1], sem_w.at[i])

    def qkv_copy(m, q):
        cols = pl.ds(256 * q, 256)
        return pltpu.make_async_copy(wqkv[m][0].at[:, cols], wqkv[m][1].at[:, cols], sem_q.at[m, q])

    def x_copy(i):
        return pltpu.make_async_copy(x_hbm.at[pl.ds(i * L, L)], xio.at[pl.ds(i * L, L)], sem_x.at[i])

    def x0_copy(i):
        r = pl.ds(pl.multiple_of(i * 128, 128), 128)
        return pltpu.make_async_copy(x_hbm.at[r], xio.at[r], sem_x0.at[i])

    def o_copy(i):
        r = pl.multiple_of(i * BM, BM)
        return pltpu.make_async_copy(xio.at[pl.ds(r, BM)], out_hbm.at[pl.ds(r, BM)], sem_o.at[i])

    b_copy = pltpu.make_async_copy(beta_hbm, bt, sem_b)
    for i in range(4):
        x0_copy(i).start()
    qkv_copy(0, 0).start()
    qkv_copy(1, 0).start()
    b_copy.start()
    hb[0:8, :] = jnp.zeros((8, D), f32)
    hb[8 + S_LEN:16 + S_LEN, :] = jnp.zeros((8, D), f32)

    def unit(u):
        return u // G, u % G

    def xs_of(s):
        return i2b(xn[pl.ds(pl.multiple_of(s * (L // 2), L // 2), L // 2), :])

    def col(g):
        return pl.ds(pl.multiple_of(g * 128, 128), 128)

    def rows64(c):
        return pl.ds(pl.multiple_of(c * 64, 64), 64), pl.ds(pl.multiple_of(c * 32, 32), 32)

    def rowsn(c, n):
        return pl.ds(pl.multiple_of(c * n, n), n), pl.ds(pl.multiple_of(c * (n // 2), n // 2), n // 2)

    def XN(c, rep, n=64):
        r, rp = rowsn(c, n)
        x = jnp.where(rep == 0, xio[r, :].astype(f32), xf[r, :])
        xf[r, :] = x
        xn[rp, :] = b2i(_ln(x).astype(bf16))

    def LNLN(c, n=64):
        r, rp = rowsn(c, n)
        z, y = _ln2(xf[r, :])
        zf[r, :] = z
        y1[rp, :] = b2i(y.astype(bf16))

    def D1q(u):
        s, g = unit(u)
        q = _dot(xs_of(s), wq[:, col(g)])
        qs[...] = b2i((q * QSCALE).astype(bf16))
        pq[u % 4] = b2i(_phi(q).astype(bf16))

    def D1k(u):
        s, g = unit(u)
        k = _dot(xs_of(s), wk[:, col(g)])
        kb[...] = b2i(k.astype(bf16))
        pk[u % 4] = b2i(_phi(k).astype(bf16))

    def D1v(u):
        s, g = unit(u)
        v = _dot(xs_of(s), wv[:, col(g)])
        vt[...] = b2i(v.astype(bf16).T)

    def S_stage(j):
        n = 128 * (j + 1)
        lane = lax.broadcasted_iota(i32, (64, 128), 1)
        hm = [jnp.where((lane >= 32 * h) & (lane < 32 * h + 32), -1, 0).astype(i32) for h in range(4)]
        valid = lax.broadcasted_iota(i32, (128, 128), 0) <= lax.broadcasted_iota(i32, (128, 128), 1)
        k4 = i2b(kb[:n // 2, :])
        qj = qs[64 * j:64 * j + 64, :]
        qst = i2b(jnp.concatenate([qj & hm[h] for h in range(4)], axis=0))
        sT = lax.dot_general(k4, qst, NT, preferred_element_type=f32)
        for h in range(4):
            sh = sT[:, 128 * h:128 * h + 128]
            dg = jnp.where(valid, sh[128 * j:], NEG)
            sh = jnp.concatenate([sh[:128 * j], dg], axis=0) if j else dg
            sb[OFF[j]:OFF[j] + n, 128 * h:128 * h + 128] = sh
            m = jnp.max(sh, axis=0, keepdims=True)
            mb[8 * j:8 * j + 8, 128 * h:128 * h + 128] = jnp.broadcast_to(m, (8, 128))

    def E_stage(j, u):
        s_, g = unit(u)
        ps, rs = [], []
        for h in range(4):
            m = mb[8 * j:8 * j + 8, 128 * h:128 * h + 128]
            l = None
            pt = []
            for i in range(j + 1):
                r0 = OFF[j] + 128 * i
                s = sb[r0:r0 + 128, 128 * h:128 * h + 128]
                p = jnp.exp2(s.reshape(16, 8, 128) - m[None])
                li = jnp.sum(p, axis=0)
                l = li if l is None else l + li
                pt.append(p.reshape(128, 128).astype(bf16))
            lt = jnp.sum(l, axis=0, keepdims=True)
            rs.append(jnp.broadcast_to(1.0 / lt, (8, 128)) * (1.0 - gate8(g, h)))
            ps.append(pt)
        return ps, rs

    def gate8(g, h):
        return gt[pl.ds(pl.multiple_of(g * 32 + 8 * h, 8), 8), :]

    def V_dots(j, ps, rs):
        outs = []
        for h in range(4):
            acc = None
            for i in range(j + 1):
                vh = i2b(vt[16 * h:16 * h + 16, 128 * i:128 * i + 128])
                d = _dot(vh, ps[h][i])
                acc = d if acc is None else acc + d
            outs.append((acc.reshape(4, 8, 128) * rs[h][None]).reshape(32, 128))
        return jnp.concatenate(outs, axis=0)

    def M_read(u):
        s, g = unit(u)
        mtb = mt[g].astype(bf16)
        nd = lax.dot_general(mtb, i2b(pq[u % 4]), NT, preferred_element_type=f32)
        outs = []
        for h in range(4):
            den = jnp.broadcast_to(nd[128 + h:129 + h], (8, 512)) + 1e-6
            c = jnp.concatenate([gate8(g, h)] * 4, axis=1) / den
            outs.append((nd[32 * h:32 * h + 32].reshape(4, 8, 512) * c[None]).reshape(32, 512))
        return jnp.concatenate(outs, axis=0)

    def V_finish(u, adots, amem):
        s, g = unit(u)
        o = jnp.concatenate(adots, axis=1)
        if amem is not None:
            o = o + amem
        ob[pl.ds(pl.multiple_of(s * 256, 256), 256), col(g)] = b2i(o.astype(bf16).T)

    def M_update(u, first_seg):
        s, g = unit(u)
        ones = jnp.full((8, 512), 0x3F803F80, i32)
        lhs = i2b(jnp.concatenate([vt[...], ones], axis=0))
        upd = _dot(lhs, i2b(pk[u % 4]))
        r = lax.broadcasted_iota(i32, (144, 128), 0)
        c = lax.broadcasted_iota(i32, (144, 128), 1)
        rh = jnp.where(r < 128, r // 32, r - 128)
        upd = jnp.where(rh == c // 32, upd, 0.0)
        if first_seg:
            mt[g] = upd
        else:
            mt[g] = mt[g] + upd

    def D2(v):
        s, c = unit(v)
        o = i2b(ob[pl.ds(pl.multiple_of(s * 256, 256), 256), :])
        y = _dot(o, wo[:, col(c)])
        rows = pl.ds(pl.multiple_of(s * L, L), L)
        xf[rows, col(c)] = xf[rows, col(c)] + y

    def a_iter(t, rep, on, first_seg=False, order="order1"):
        adots = [None] * 4
        pr = [None] * 4
        amem = None
        for tok in cfg[order].split():
            k = tok[0]
            if k not in on:
                continue
            if k == "V":
                adots[int(tok[1])] = V_dots(int(tok[1]), *pr[int(tok[1])])
            elif k == "E":
                pr[int(tok[1])] = E_stage(int(tok[1]), t)
            elif k == "S":
                S_stage(int(tok[1]))
            elif k == "D":
                D2(t - 8)
            elif k == "X":
                XN(jnp.minimum(t + 10, 31), rep)
            elif k == "N":
                LNLN(jnp.maximum(t - 16, 0))
            elif k == "R":
                if not first_seg:
                    amem = M_read(t)
            elif k == "F":
                V_finish(t, adots, amem)
            elif k == "U":
                M_update(t, first_seg)
            elif k == "Q":
                D1q(t + 2)
            elif k == "K":
                D1k(t + 2)
            elif k == "W":
                D1v(t + 1)

    def B1(i, half):
        lhs = i2b(y1[pl.ds(pl.multiple_of(i * (BM // 2), BM // 2), BM // 2), :])
        cols = slice(512 * half, 512 * half + 512)
        hb[pl.ds(pl.multiple_of(i * BM + 8, 8), BM), cols] = _gelu(_dot(lhs, w1[:, cols]))

    def shifted(r0):
        win_ = hb[pl.ds(pl.multiple_of(r0, 8), 144), :]
        parts = []
        for gi, sh in enumerate((-1, 1, -2, 2)):
            parts.append(win_[8 + sh:8 + sh + 128, 256 * gi:256 * gi + 256])
        return jnp.concatenate(parts, axis=1).astype(bf16)

    def bb_body(i, rep):
        rows = [pl.multiple_of(i * BM + 128 * a, 128) for a in range(2)]
        x1 = [zf[pl.ds(r, 128), :] + _dot(shifted(r), w2[...]) for r in rows]
        y2 = [_ln(v).astype(bf16) for v in x1]
        gg = [_gelu(_dot(y2[a], w3[...])).astype(bf16) for a in range(2)]
        for a in range(2):
            r = rows[a]
            xo = xf[pl.ds(r, 128), :] + x1[a] + _dot(gg[a], w4[...])
            xf[pl.ds(r, 128), :] = xo
            xio[pl.ds(r, 128), :] = xo.astype(bf16)

        @pl.when(rep == 1)
        def _():
            o_copy(i).start()
        return rep

    ALL = "VESDXNRFUQKW"

    def l1(t, rep):
        for tt, wi in ((2, 0), (4, 1), (6, 2)):
            @pl.when((rep == 0) & (t == tt))
            def _():
                w_copy(wi).start()
        for tt, q in ((2, 2), (4, 3)):
            @pl.when((rep == 0) & (t == tt))
            def _():
                for m in range(3):
                    qkv_copy(m, q).wait()

        @pl.when((rep == 0) & (t == 6))
        def _():
            x_copy(2).wait()
        a_iter(t, rep, "VESXRFUQKW", first_seg=True)
        return rep

    def l2(t, rep):
        for tt, wi in ((11, 3), (16, 4)):
            @pl.when((rep == 0) & (t == tt))
            def _():
                w_copy(wi).start()

        @pl.when((rep == 0) & (t == 14))
        def _():
            x_copy(3).wait()
        a_iter(t, rep, ALL, order="order2")
        return rep

    if cfg["mode"] == "l2":
        lax.fori_loop(8, 30, l2, 0)
        return
    if cfg["mode"] == "l1":
        lax.fori_loop(0, 8, l1, 0)
        return
    if cfg["mode"] == "bb":
        lax.fori_loop(0, NB, bb_body, 0)
        return

    def rep_body(rep, c):
        with scope("z_xn0"):
            def xn0(c_, carry):
                @pl.when(rep == 0)
                def _():
                    x0_copy(c_).wait()

                @pl.when((rep == 0) & (c_ == 1))
                def _():
                    x_copy(1).start()
                    qkv_copy(2, 0).start()
                XN(c_, rep, 128)
                return carry
            lax.fori_loop(0, 4, xn0, 0)

            @pl.when(rep == 0)
            def _():
                b_copy.wait()
                hr = lax.broadcasted_iota(i32, (H * 8, H), 0) // 8
                hc = lax.broadcasted_iota(i32, (H * 8, H), 1)
                bsel = jnp.sum(jnp.where(hr == hc, bt[...].astype(f32), 0.0), axis=1, keepdims=True)
                gt[...] = jnp.broadcast_to(jax.nn.sigmoid(bsel), (H * 8, 128))

        with scope("z_apro"):
            @pl.when(rep == 0)
            def _():
                qkv_copy(0, 0).wait()
                qkv_copy(1, 0).wait()
            a_iter(-2, rep, "QK")

            @pl.when(rep == 0)
            def _():
                x_copy(1).wait()
                qkv_copy(2, 0).wait()
                for m in range(3):
                    qkv_copy(m, 1).start()
            XN(8, rep)
            XN(9, rep)
            a_iter(-1, rep, "SWQK")

            @pl.when(rep == 0)
            def _():
                for m in range(3):
                    qkv_copy(m, 1).wait()
                for q in (2, 3):
                    for m in range(3):
                        qkv_copy(m, q).start()
                x_copy(2).start()
                x_copy(3).start()

        with scope("z_l1"):
            lax.fori_loop(0, 8, l1, rep)

        @pl.when(rep == 0)
        def _():
            w_copy(0).wait()

        with scope("z_l2"):
            lax.fori_loop(8, 30, l2, rep)
        with scope("z_aepi"):
            a_iter(30, rep, "VESDNRFW", order="order3")
            a_iter(31, rep, "VEDNRF", order="order3")

        @pl.when(rep == 0)
        def _():
            for i in range(1, 5):
                w_copy(i).wait()

        def t1(i, c):
            for tok in cfg["order4"].split():
                if tok[0] == "D":
                    D2(24 + 2 * i + int(tok[1]))
                elif tok[0] == "N":
                    LNLN(8 + i, 128)
                else:
                    B1(i, int(tok[1]))
            return c

        def t2(i, c):
            for tok in cfg["order5"].split():
                if tok[0] == "N":
                    LNLN(jnp.minimum(12 + 2 * (i - 4) + int(tok[1]), 15), 128)
                else:
                    B1(i, int(tok[1]))
            return c
        with scope("z_t1"):
            lax.fori_loop(0, 4, t1, 0)
        with scope("z_t2"):
            lax.fori_loop(4, 8, t2, 0)
        if cfg["mode"] != "A":
            with scope("z_bb"):
                lax.fori_loop(0, NB, bb_body, rep)
        return c

    lax.fori_loop(0, 2, rep_body, 0)
    with scope("z_owait"):
        for i in range(NB):
            o_copy(i).wait()


def build(cfg, name="infini_mixer"):
    vm = pltpu.VMEM
    scratch = [
        vm((S_LEN, D), bf16),
        vm((D, D), bf16), vm((D, D), bf16), vm((D, D), bf16), vm((D, D), bf16),
        vm((D, D), bf16), vm((D, D), bf16), vm((D, F), bf16), vm((F, D), bf16),
        vm((S_LEN, D), f32),
        vm((S_LEN, D), f32),
        vm((S_LEN // 2, D), i32),
        vm((S_LEN // 2, D), i32),
        vm((256, 128), i32), vm((256, 128), i32),
        vm((4, 256, 128), i32), vm((4, 256, 128), i32),
        vm((64, 512), i32),
        vm((1280, 512), f32), vm((32, 512), f32),
        vm((S_LEN // 2, D), i32),
        vm((G, 144, 128), f32),
        vm((S_LEN + 16, D), f32),
        vm((H * 8, 128), f32), vm((1, H), bf16),
        pltpu.SemaphoreType.DMA((4,)), pltpu.SemaphoreType.DMA((3, 4)),
        pltpu.SemaphoreType.DMA((5,)), pltpu.SemaphoreType.DMA((NB,)), pltpu.SemaphoreType.DMA(()),
        pltpu.SemaphoreType.DMA((4,)),
    ]
    any_spec = pl.BlockSpec(memory_space=pl.ANY)
    return pl.pallas_call(
        functools.partial(_kernel, cfg=cfg),
        out_shape=jax.ShapeDtypeStruct((S_LEN, D), bf16),
        in_specs=[any_spec] * 10,
        out_specs=any_spec,
        scratch_shapes=scratch,
        compiler_params=pltpu.CompilerParams(vmem_limit_bytes=110 * 2 ** 20),
        name=name,
    )


def make_kernel(cfg, name="infini_mixer"):
    def pallas_interleave_layers__memory_aug_infini_attn__mixer_s_mlp__prompt_kernel(A_x, A_wq, A_wk, A_wv, A_wo, A_beta, B_x, B_w1, B_w2, B_w3, B_w4):
        beta = A_beta.reshape(1, H)
        out = build(cfg, name)(A_x.reshape(S_LEN, D), A_wq, A_wk, A_wv, A_wo, beta, B_w1, B_w2, B_w3, B_w4)
        return out.reshape(1, S_LEN, D)
    return jax.jit(kernel)


kernel = make_kernel(CFG)
```

```python
import functools
import math

import numpy as np
import jax
import jax.numpy as jnp
from jax import lax
import jax.experimental.pallas as pl
import jax.experimental.pallas.tpu as pltpu

S_LEN = 2048
D = 1024
F = 3584
H = 32
DH = 32
NSEG = 4
L = 512
G = 8
NU = NSEG * G
OFF = (0, 128, 384, 768)
EPS = 1e-5
QSCALE = float(DH ** -0.5 * math.log2(math.e))
NEG = -1e30
BM = 256
NB = S_LEN // BM

f32 = jnp.float32
bf16 = jnp.bfloat16
i32 = jnp.int32
NT = (((1,), (1,)), ((), ()))

CONSTRAINTS = [("E.", "V#"), ("E.", "S#"), ("V.", "W"), ("U", "W"), ("S.", "Q"), ("S.", "K"), ("R", "U"), ("V.", "F"), ("R", "F")]
SEARCH_MODE = "A"
SEARCH_T = 400.0


def score(loops, total):
    rep, xn0, l1, l2, t1, t2 = loops[:6]
    ln = lambda x: x[1] - x[0]
    straight = ln(rep) - ln(xn0) - ln(l1) - ln(l2) - ln(t1) - ln(t2)
    parts = [ln(xn0), ln(l1), ln(l2), ln(t1), ln(t2), straight]
    return 4 * ln(xn0) + 8 * ln(l1) + 22 * ln(l2) + 4 * ln(t1) + 4 * ln(t2) + straight, parts


COMPONENTS = {"order1": (lambda p: p[1], 25.0), "order2": (lambda p: p[2], 25.0), "order3": (lambda p: p[5], 30.0),
              "order4": (lambda p: p[3], 30.0), "order5": (lambda p: p[4], 30.0)}
CFG = dict(
    order1="E1 E0 S0 V0 E2 E3 R N S2 V2 S3 S1 K V3 V1 D U W Q X F",
    order2="E0 E1 X E3 S3 V0 S0 S1 V1 E2 S2 R D K V3 V2 U W Q N F",
    order3="E1 E3 S1 E0 E2 S0 V1 S3 V3 X S2 V2 V0 Q R K U F W D N",
    order4="B0 N B1 D0 D1",
    order5="B0 N0 B1 N1",
    mode="full",
    scopes=False,
)


def i2b(x):
    return pltpu.bitcast(x, bf16)


def b2i(x):
    return pltpu.bitcast(x, i32)


def _ln(x):
    m = jnp.mean(x, axis=-1, keepdims=True)
    d = x - m
    v = jnp.mean(d * d, axis=-1, keepdims=True)
    return d * lax.rsqrt(v + EPS)


def _ln2(x):
    m = jnp.mean(x, axis=-1, keepdims=True)
    d = x - m
    v = jnp.mean(d * d, axis=-1, keepdims=True)
    r = lax.rsqrt(v + EPS)
    r2 = r * lax.rsqrt(v * r * r + EPS)
    return d * r, d * r2


def _gelu(x):
    c0 = math.sqrt(2.0 / math.pi)
    c1 = c0 * 0.044715
    return (0.5 * x) * (1.0 + jnp.tanh(x * (c0 + c1 * (x * x))))


def _phi(t):
    return jnp.where(t > 0, t + 1.0, jnp.exp(t))


def _dot(a, b):
    return jnp.dot(a, b, preferred_element_type=f32)


class _NoScope:
    def __enter__(self):
        return self

    def __exit__(self, *a):
        return False


def _kernel(x_hbm, wq_hbm, wk_hbm, wv_hbm, wo_hbm, beta_hbm, w1_hbm, w2_hbm, w3_hbm, w4_hbm,
            out_hbm,
            xio, wq, wk, wv, wo, w1, w2, w3, w4,
            xf, zf, xn, y1, qs, kb, pq, pk, vt, sb, mb, ob, mt, hb, gt, bt,
            sem_x, sem_q, sem_w, sem_o, sem_b, sem_x0, *, cfg):
    scope = jax.named_scope if cfg["scopes"] else (lambda name: _NoScope())
    wlate = [(wo_hbm, wo), (w1_hbm, w1), (w2_hbm, w2), (w3_hbm, w3), (w4_hbm, w4)]
    wqkv = [(wq_hbm, wq), (wk_hbm, wk), (wv_hbm, wv)]

    def w_copy(i):
        return pltpu.make_async_copy(wlate[i][0], wlate[i][1], sem_w.at[i])

    def qkv_copy(m, q):
        cols = pl.ds(256 * q, 256)
        return pltpu.make_async_copy(wqkv[m][0].at[:, cols], wqkv[m][1].at[:, cols], sem_q.at[m, q])

    def x_copy(i):
        return pltpu.make_async_copy(x_hbm.at[pl.ds(i * L, L)], xio.at[pl.ds(i * L, L)], sem_x.at[i])

    def x0_copy(i):
        r = pl.ds(pl.multiple_of(i * 128, 128), 128)
        return pltpu.make_async_copy(x_hbm.at[r], xio.at[r], sem_x0.at[i])

    def o_copy(i):
        r = pl.multiple_of(i * BM, BM)
        return pltpu.make_async_copy(xio.at[pl.ds(r, BM)], out_hbm.at[pl.ds(r, BM)], sem_o.at[i])

    b_copy = pltpu.make_async_copy(beta_hbm, bt, sem_b)
    for i in range(4):
        x0_copy(i).start()
    qkv_copy(0, 0).start()
    qkv_copy(1, 0).start()
    b_copy.start()
    hb[0:8, :] = jnp.zeros((8, D), f32)
    hb[8 + S_LEN:16 + S_LEN, :] = jnp.zeros((8, D), f32)

    def unit(u):
        return u // G, u % G

    def xs_of(s):
        return i2b(xn[pl.ds(pl.multiple_of(s * (L // 2), L // 2), L // 2), :])

    def col(g):
        return pl.ds(pl.multiple_of(g * 128, 128), 128)

    def rows64(c):
        return pl.ds(pl.multiple_of(c * 64, 64), 64), pl.ds(pl.multiple_of(c * 32, 32), 32)

    def rowsn(c, n):
        return pl.ds(pl.multiple_of(c * n, n), n), pl.ds(pl.multiple_of(c * (n // 2), n // 2), n // 2)

    def XN(c, rep, n=64):
        r, rp = rowsn(c, n)
        x = jnp.where(rep == 0, xio[r, :].astype(f32), xf[r, :])
        xf[r, :] = x
        xn[rp, :] = b2i(_ln(x).astype(bf16))

    def LNLN(c, n=64):
        r, rp = rowsn(c, n)
        z, y = _ln2(xf[r, :])
        zf[r, :] = z
        y1[rp, :] = b2i(y.astype(bf16))

    def D1q(u):
        s, g = unit(u)
        q = _dot(xs_of(s), wq[:, col(g)])
        qs[...] = b2i((q * QSCALE).astype(bf16))
        pq[u % 4] = b2i(_phi(q).astype(bf16))

    def D1k(u):
        s, g = unit(u)
        k = _dot(xs_of(s), wk[:, col(g)])
        kb[...] = b2i(k.astype(bf16))
        pk[u % 4] = b2i(_phi(k).astype(bf16))

    def D1v(u):
        s, g = unit(u)
        v = _dot(xs_of(s), wv[:, col(g)])
        vt[...] = b2i(v.astype(bf16).T)

    def S_stage(j):
        n = 128 * (j + 1)
        lane = lax.broadcasted_iota(i32, (64, 128), 1)
        hm = [jnp.where((lane >= 32 * h) & (lane < 32 * h + 32), -1, 0).astype(i32) for h in range(4)]
        valid = lax.broadcasted_iota(i32, (128, 128), 0) <= lax.broadcasted_iota(i32, (128, 128), 1)
        k4 = i2b(kb[:n // 2, :])
        qj = qs[64 * j:64 * j + 64, :]
        qst = i2b(jnp.concatenate([qj & hm[h] for h in range(4)], axis=0))
        sT = lax.dot_general(k4, qst, NT, preferred_element_type=f32)
        for h in range(4):
            sh = sT[:, 128 * h:128 * h + 128]
            dg = jnp.where(valid, sh[128 * j:], NEG)
            sh = jnp.concatenate([sh[:128 * j], dg], axis=0) if j else dg
            sb[OFF[j]:OFF[j] + n, 128 * h:128 * h + 128] = sh
            m = jnp.max(sh, axis=0, keepdims=True)
            mb[8 * j:8 * j + 8, 128 * h:128 * h + 128] = jnp.broadcast_to(m, (8, 128))

    def E_stage(j, u):
        s_, g = unit(u)
        ps, rs = [], []
        for h in range(4):
            m = mb[8 * j:8 * j + 8, 128 * h:128 * h + 128]
            l = None
            pt = []
            for i in range(j + 1):
                r0 = OFF[j] + 128 * i
                s = sb[r0:r0 + 128, 128 * h:128 * h + 128]
                p = jnp.exp2(s.reshape(16, 8, 128) - m[None])
                li = jnp.sum(p, axis=0)
                l = li if l is None else l + li
                pt.append(p.reshape(128, 128).astype(bf16))
            lt = jnp.sum(l, axis=0, keepdims=True)
            rs.append(jnp.broadcast_to(1.0 / lt, (8, 128)) * (1.0 - gate8(g, h)))
            ps.append(pt)
        return ps, rs

    def gate8(g, h):
        return gt[pl.ds(pl.multiple_of(g * 32 + 8 * h, 8), 8), :]

    def V_dots(j, ps, rs):
        outs = []
        for h in range(4):
            acc = None
            for i in range(j + 1):
                vh = i2b(vt[16 * h:16 * h + 16, 128 * i:128 * i + 128])
                d = _dot(vh, ps[h][i])
                acc = d if acc is None else acc + d
            outs.append((acc.reshape(4, 8, 128) * rs[h][None]).reshape(32, 128))
        return jnp.concatenate(outs, axis=0)

    def M_read(u):
        s, g = unit(u)
        mtb = mt[g].astype(bf16)
        nd = lax.dot_general(mtb, i2b(pq[u % 4]), NT, preferred_element_type=f32)
        outs = []
        for h in range(4):
            den = jnp.broadcast_to(nd[128 + h:129 + h], (8, 512)) + 1e-6
            c = jnp.concatenate([gate8(g, h)] * 4, axis=1) / den
            outs.append((nd[32 * h:32 * h + 32].reshape(4, 8, 512) * c[None]).reshape(32, 512))
        return jnp.concatenate(outs, axis=0)

    def V_finish(u, adots, amem):
        s, g = unit(u)
        o = jnp.concatenate(adots, axis=1)
        if amem is not None:
            o = o + amem
        ob[pl.ds(pl.multiple_of(s * 256, 256), 256), col(g)] = b2i(o.astype(bf16).T)

    def M_update(u, first_seg):
        s, g = unit(u)
        ones = jnp.full((8, 512), 0x3F803F80, i32)
        lhs = i2b(jnp.concatenate([vt[...], ones], axis=0))
        upd = _dot(lhs, i2b(pk[u % 4]))
        r = lax.broadcasted_iota(i32, (144, 128), 0)
        c = lax.broadcasted_iota(i32, (144, 128), 1)
        rh = jnp.where(r < 128, r // 32, r - 128)
        upd = jnp.where(rh == c // 32, upd, 0.0)
        if first_seg:
            mt[g] = upd
        else:
            mt[g] = mt[g] + upd

    def D2(v):
        s, c = unit(v)
        o = i2b(ob[pl.ds(pl.multiple_of(s * 256, 256), 256), :])
        y = _dot(o, wo[:, col(c)])
        rows = pl.ds(pl.multiple_of(s * L, L), L)
        xf[rows, col(c)] = xf[rows, col(c)] + y

    def a_iter(t, rep, on, first_seg=False, order="order1"):
        adots = [None] * 4
        pr = [None] * 4
        amem = None
        for tok in cfg[order].split():
            k = tok[0]
            if k not in on:
                continue
            if k == "V":
                adots[int(tok[1])] = V_dots(int(tok[1]), *pr[int(tok[1])])
            elif k == "E":
                pr[int(tok[1])] = E_stage(int(tok[1]), t)
            elif k == "S":
                S_stage(int(tok[1]))
            elif k == "D":
                D2(t - 8)
            elif k == "X":
                XN(jnp.minimum(t + 10, 31), rep)
            elif k == "N":
                LNLN(jnp.maximum(t - 16, 0))
            elif k == "R":
                if not first_seg:
                    amem = M_read(t)
            elif k == "F":
                V_finish(t, adots, amem)
            elif k == "U":
                M_update(t, first_seg)
            elif k == "Q":
                D1q(t + 2)
            elif k == "K":
                D1k(t + 2)
            elif k == "W":
                D1v(t + 1)

    def B1(i, half):
        lhs = i2b(y1[pl.ds(pl.multiple_of(i * (BM // 2), BM // 2), BM // 2), :])
        cols = slice(512 * half, 512 * half + 512)
        hb[pl.ds(pl.multiple_of(i * BM + 8, 8), BM), cols] = _gelu(_dot(lhs, w1[:, cols]))

    def shifted(r0):
        win_ = hb[pl.ds(pl.multiple_of(r0, 8), 144), :]
        parts = []
        for gi, sh in enumerate((-1, 1, -2, 2)):
            parts.append(win_[8 + sh:8 + sh + 128, 256 * gi:256 * gi + 256])
        return jnp.concatenate(parts, axis=1).astype(bf16)

    def bb_body(i, rep):
        rows = [pl.multiple_of(i * BM + 128 * a, 128) for a in range(2)]
        x1 = [zf[pl.ds(r, 128), :] + _dot(shifted(r), w2[...]) for r in rows]
        y2 = [_ln(v).astype(bf16) for v in x1]
        gg = [_gelu(_dot(y2[a], w3[...])).astype(bf16) for a in range(2)]
        for a in range(2):
            r = rows[a]
            xo = xf[pl.ds(r, 128), :] + x1[a] + _dot(gg[a], w4[...])
            xf[pl.ds(r, 128), :] = xo
            xio[pl.ds(r, 128), :] = xo.astype(bf16)

        @pl.when(rep == 1)
        def _():
            o_copy(i).start()
        return rep

    ALL = "VESDXNRFUQKW"

    def l1(t, rep):
        for tt, wi in ((2, 0), (4, 1), (6, 2)):
            @pl.when((rep == 0) & (t == tt))
            def _():
                w_copy(wi).start()
        for tt, q in ((2, 2), (4, 3)):
            @pl.when((rep == 0) & (t == tt))
            def _():
                for m in range(3):
                    qkv_copy(m, q).wait()

        @pl.when((rep == 0) & (t == 6))
        def _():
            x_copy(2).wait()
        a_iter(t, rep, "VESXRFUQKW", first_seg=True)
        return rep

    def l2(t, rep):
        for tt, wi in ((11, 3), (16, 4)):
            @pl.when((rep == 0) & (t == tt))
            def _():
                w_copy(wi).start()

        @pl.when((rep == 0) & (t == 14))
        def _():
            x_copy(3).wait()
        a_iter(t, rep, ALL, order="order2")
        return rep

    if cfg["mode"] == "l2":
        lax.fori_loop(8, 30, l2, 0)
        return
    if cfg["mode"] == "l1":
        lax.fori_loop(0, 8, l1, 0)
        return
    if cfg["mode"] == "bb":
        lax.fori_loop(0, NB, bb_body, 0)
        return

    def rep_body(rep, c):
        with scope("z_xn0"):
            def xn0(c_, carry):
                @pl.when(rep == 0)
                def _():
                    x0_copy(c_).wait()

                @pl.when((rep == 0) & (c_ == 1))
                def _():
                    x_copy(1).start()
                    qkv_copy(2, 0).start()
                XN(c_, rep, 128)
                return carry
            lax.fori_loop(0, 4, xn0, 0)

            @pl.when(rep == 0)
            def _():
                b_copy.wait()
                hr = lax.broadcasted_iota(i32, (H * 8, H), 0) // 8
                hc = lax.broadcasted_iota(i32, (H * 8, H), 1)
                bsel = jnp.sum(jnp.where(hr == hc, bt[...].astype(f32), 0.0), axis=1, keepdims=True)
                gt[...] = jnp.broadcast_to(jax.nn.sigmoid(bsel), (H * 8, 128))

        with scope("z_apro"):
            @pl.when(rep == 0)
            def _():
                qkv_copy(0, 0).wait()
                qkv_copy(1, 0).wait()
            a_iter(-2, rep, "QK")

            @pl.when(rep == 0)
            def _():
                x_copy(1).wait()
                qkv_copy(2, 0).wait()
                for m in range(3):
                    qkv_copy(m, 1).start()
            XN(8, rep)
            XN(9, rep)
            a_iter(-1, rep, "SWQK")

            @pl.when(rep == 0)
            def _():
                for m in range(3):
                    qkv_copy(m, 1).wait()
                for q in (2, 3):
                    for m in range(3):
                        qkv_copy(m, q).start()
                x_copy(2).start()
                x_copy(3).start()

        with scope("z_l1"):
            lax.fori_loop(0, 8, l1, rep)

        @pl.when(rep == 0)
        def _():
            w_copy(0).wait()

        with scope("z_l2"):
            lax.fori_loop(8, 30, l2, rep)
        with scope("z_aepi"):
            a_iter(30, rep, "VESDNRFW", order="order3")
            a_iter(31, rep, "VEDNRF", order="order3")

        @pl.when(rep == 0)
        def _():
            for i in range(1, 5):
                w_copy(i).wait()

        def t1(i, c):
            for tok in cfg["order4"].split():
                if tok[0] == "D":
                    D2(24 + 2 * i + int(tok[1]))
                elif tok[0] == "N":
                    LNLN(8 + i, 128)
                else:
                    B1(i, int(tok[1]))
            return c

        def t2(i, c):
            for tok in cfg["order5"].split():
                if tok[0] == "N":
                    LNLN(jnp.minimum(12 + 2 * (i - 4) + int(tok[1]), 15), 128)
                else:
                    B1(i, int(tok[1]))
            return c
        with scope("z_t1"):
            lax.fori_loop(0, 4, t1, 0)
        with scope("z_t2"):
            lax.fori_loop(4, 8, t2, 0)
        if cfg["mode"] != "A":
            with scope("z_bb"):
                lax.fori_loop(0, NB, bb_body, rep)
        return c

    lax.fori_loop(0, 2, rep_body, 0)
    with scope("z_owait"):
        for i in range(NB):
            o_copy(i).wait()


def build(cfg, name="infini_mixer"):
    vm = pltpu.VMEM
    scratch = [
        vm((S_LEN, D), bf16),
        vm((D, D), bf16), vm((D, D), bf16), vm((D, D), bf16), vm((D, D), bf16),
        vm((D, D), bf16), vm((D, D), bf16), vm((D, F), bf16), vm((F, D), bf16),
        vm((S_LEN, D), f32),
        vm((S_LEN, D), f32),
        vm((S_LEN // 2, D), i32),
        vm((S_LEN // 2, D), i32),
        vm((256, 128), i32), vm((256, 128), i32),
        vm((4, 256, 128), i32), vm((4, 256, 128), i32),
        vm((64, 512), i32),
        vm((1280, 512), f32), vm((32, 512), f32),
        vm((S_LEN // 2, D), i32),
        vm((G, 144, 128), f32),
        vm((S_LEN + 16, D), f32),
        vm((H * 8, 128), f32), vm((1, H), bf16),
        pltpu.SemaphoreType.DMA((4,)), pltpu.SemaphoreType.DMA((3, 4)),
        pltpu.SemaphoreType.DMA((5,)), pltpu.SemaphoreType.DMA((NB,)), pltpu.SemaphoreType.DMA(()),
        pltpu.SemaphoreType.DMA((4,)),
    ]
    any_spec = pl.BlockSpec(memory_space=pl.ANY)
    return pl.pallas_call(
        functools.partial(_kernel, cfg=cfg),
        out_shape=jax.ShapeDtypeStruct((S_LEN, D), bf16),
        in_specs=[any_spec] * 10,
        out_specs=any_spec,
        scratch_shapes=scratch,
        compiler_params=pltpu.CompilerParams(vmem_limit_bytes=110 * 2 ** 20),
        name=name,
    )


def make_kernel(cfg, name="infini_mixer"):
    def pallas_interleave_layers__memory_aug_infini_attn__mixer_s_mlp__prompt_kernel(A_x, A_wq, A_wk, A_wv, A_wo, A_beta, B_x, B_w1, B_w2, B_w3, B_w4):
        beta = A_beta.reshape(1, H)
        out = build(cfg, name)(A_x.reshape(S_LEN, D), A_wq, A_wk, A_wv, A_wo, beta, B_w1, B_w2, B_w3, B_w4)
        return out.reshape(1, S_LEN, D)
    return jax.jit(kernel)


kernel = make_kernel(CFG)
```

```python
import functools
import math

import numpy as np
import jax
import jax.numpy as jnp
from jax import lax
import jax.experimental.pallas as pl
import jax.experimental.pallas.tpu as pltpu

S_LEN = 2048
D = 1024
F = 3584
H = 32
DH = 32
NSEG = 4
L = 512
G = 8
NU = NSEG * G
OFF = (0, 128, 384, 768)
EPS = 1e-5
QSCALE = float(DH ** -0.5 * math.log2(math.e))
NEG = -1e30
BM = 256
NB = S_LEN // BM

f32 = jnp.float32
bf16 = jnp.bfloat16
i32 = jnp.int32
NT = (((1,), (1,)), ((), ()))

CONSTRAINTS = [("E.", "V#"), ("E.", "S#"), ("V.", "W"), ("U", "W"), ("S.", "Q"), ("S.", "K"), ("R", "U"), ("V.", "F"), ("R", "F")]
SEARCH_MODE = "A"
SEARCH_T = 400.0


def score(loops, total):
    rep, xn0, l1, l2, t1, t2 = loops[:6]
    ln = lambda x: x[1] - x[0]
    straight = ln(rep) - ln(xn0) - ln(l1) - ln(l2) - ln(t1) - ln(t2)
    parts = [ln(xn0), ln(l1), ln(l2), ln(t1), ln(t2), straight]
    return 4 * ln(xn0) + 8 * ln(l1) + 22 * ln(l2) + 4 * ln(t1) + 4 * ln(t2) + straight, parts


COMPONENTS = {"order1": (lambda p: p[1], 25.0), "order2": (lambda p: p[2], 25.0), "order3": (lambda p: p[5], 30.0),
              "order4": (lambda p: p[3], 30.0), "order5": (lambda p: p[4], 30.0)}
CFG = dict(
    order1="R E0 V0 U N E1 V1 E2 S0 S2 E3 V2 S3 V3 F S1 Q W D X K",
    order2="E0 E3 S3 E2 V0 E1 S1 V1 S2 S0 R K V3 V2 U W N Q F X D",
    order3="E1 S1 E3 X E0 S0 E2 S3 V3 S2 V2 K V1 V0 R U Q F W D N",
    order4="B0 N B1 D0 D1",
    order5="B0 N0 B1 N1",
    mode="full",
    scopes=False,
)


def i2b(x):
    return pltpu.bitcast(x, bf16)


def b2i(x):
    return pltpu.bitcast(x, i32)


def _ln(x):
    m = jnp.mean(x, axis=-1, keepdims=True)
    d = x - m
    v = jnp.mean(d * d, axis=-1, keepdims=True)
    return d * lax.rsqrt(v + EPS)


def _ln2(x):
    m = jnp.mean(x, axis=-1, keepdims=True)
    d = x - m
    v = jnp.mean(d * d, axis=-1, keepdims=True)
    r = lax.rsqrt(v + EPS)
    r2 = r * lax.rsqrt(v * r * r + EPS)
    return d * r, d * r2


def _gelu(x):
    c0 = math.sqrt(2.0 / math.pi)
    c1 = c0 * 0.044715
    return (0.5 * x) * (1.0 + jnp.tanh(x * (c0 + c1 * (x * x))))


def _phi(t):
    return jnp.where(t > 0, t + 1.0, jnp.exp(t))


def _dot(a, b):
    return jnp.dot(a, b, preferred_element_type=f32)


class _NoScope:
    def __enter__(self):
        return self

    def __exit__(self, *a):
        return False


def _kernel(x_hbm, wq_hbm, wk_hbm, wv_hbm, wo_hbm, beta_hbm, w1_hbm, w2_hbm, w3_hbm, w4_hbm,
            out_hbm,
            xio, wq, wk, wv, wo, w1, w2, w3, w4,
            xf, zf, xn, y1, qs, kb, pq, pk, vt, sb, mb, ob, mt, hb, gt, bt,
            sem_x, sem_q, sem_w, sem_o, sem_b, sem_x0, *, cfg):
    scope = jax.named_scope if cfg["scopes"] else (lambda name: _NoScope())
    wlate = [(wo_hbm, wo), (w1_hbm, w1), (w2_hbm, w2), (w3_hbm, w3), (w4_hbm, w4)]
    wqkv = [(wq_hbm, wq), (wk_hbm, wk), (wv_hbm, wv)]

    def w_copy(i):
        return pltpu.make_async_copy(wlate[i][0], wlate[i][1], sem_w.at[i])

    def qkv_copy(m, q):
        cols = pl.ds(256 * q, 256)
        return pltpu.make_async_copy(wqkv[m][0].at[:, cols], wqkv[m][1].at[:, cols], sem_q.at[m, q])

    def x_copy(i):
        return pltpu.make_async_copy(x_hbm.at[pl.ds(i * L, L)], xio.at[pl.ds(i * L, L)], sem_x.at[i])

    def x0_copy(i):
        r = pl.ds(pl.multiple_of(i * 128, 128), 128)
        return pltpu.make_async_copy(x_hbm.at[r], xio.at[r], sem_x0.at[i])

    def o_copy(i):
        r = pl.multiple_of(i * BM, BM)
        return pltpu.make_async_copy(xio.at[pl.ds(r, BM)], out_hbm.at[pl.ds(r, BM)], sem_o.at[i])

    b_copy = pltpu.make_async_copy(beta_hbm, bt, sem_b)
    for i in range(4):
        x0_copy(i).start()
    qkv_copy(0, 0).start()
    qkv_copy(1, 0).start()
    b_copy.start()
    hb[0:8, :] = jnp.zeros((8, D), f32)
    hb[8 + S_LEN:16 + S_LEN, :] = jnp.zeros((8, D), f32)

    def unit(u):
        return u // G, u % G

    def xs_of(s):
        return i2b(xn[pl.ds(pl.multiple_of(s * (L // 2), L // 2), L // 2), :])

    def col(g):
        return pl.ds(pl.multiple_of(g * 128, 128), 128)

    def rows64(c):
        return pl.ds(pl.multiple_of(c * 64, 64), 64), pl.ds(pl.multiple_of(c * 32, 32), 32)

    def rowsn(c, n):
        return pl.ds(pl.multiple_of(c * n, n), n), pl.ds(pl.multiple_of(c * (n // 2), n // 2), n // 2)

    def XN(c, rep, n=64):
        r, rp = rowsn(c, n)
        x = jnp.where(rep == 0, xio[r, :].astype(f32), xf[r, :])
        xf[r, :] = x
        xn[rp, :] = b2i(_ln(x).astype(bf16))

    def LNLN(c, n=64):
        r, rp = rowsn(c, n)
        z, y = _ln2(xf[r, :])
        zf[r, :] = z
        y1[rp, :] = b2i(y.astype(bf16))

    def D1q(u):
        s, g = unit(u)
        q = _dot(xs_of(s), wq[:, col(g)])
        qs[...] = b2i((q * QSCALE).astype(bf16).T)
        pq[u % 4] = b2i(_phi(q).astype(bf16).T)

    def D1k(u):
        s, g = unit(u)
        k = _dot(xs_of(s), wk[:, col(g)])
        kb[...] = b2i(k.astype(bf16))
        pk[u % 4] = b2i(_phi(k).astype(bf16))

    def D1v(u):
        s, g = unit(u)
        v = _dot(xs_of(s), wv[:, col(g)])
        vt[...] = b2i(v.astype(bf16).T)

    def S_stage(j):
        n = 128 * j + 64
        lane = lax.broadcasted_iota(i32, (64, 128), 1)
        rr = lax.broadcasted_iota(i32, (64, 128), 0)
        valid_lo = rr <= lane
        valid_hi = rr + 64 <= lane
        qj = qs[:, 128 * j:128 * j + 128]
        z16 = jnp.zeros((16, 128), i32)
        hrows = [qj[16 * h:16 * h + 16] for h in range(4)]
        qst = jnp.concatenate(
            [jnp.concatenate([hrows[h] if r == h else z16 for r in range(4)], axis=0) for h in range(4)], axis=1)
        sT = _dot(i2b(kb[:n // 2, :]), i2b(qst))
        upper = lane[:16] >= 64
        prs = []
        for p in range(2):
            ra = jnp.where(upper, hrows[2 * p], 0)
            rb = jnp.where(upper, 0, pltpu.roll(hrows[2 * p + 1], 64, 1))
            prs.append(jnp.concatenate([(ra, rb)[r % 2] if r // 2 == p else z16 for r in range(4)], axis=0))
        sP = _dot(i2b(kb[n // 2:n // 2 + 32, :]), i2b(jnp.concatenate(prs, axis=1)))
        for h in range(4):
            sh = sT[:, 128 * h:128 * h + 128]
            hi = sP[:, 128 * (h // 2):128 * (h // 2) + 128]
            if h % 2:
                hi = pltpu.roll(hi, 64, 1)
            parts = [sh[:128 * j]] if j else []
            parts += [jnp.where(valid_lo, sh[128 * j:], NEG), jnp.where(valid_hi, hi, NEG)]
            sh = jnp.concatenate(parts, axis=0)
            sb[OFF[j]:OFF[j] + n + 64, 128 * h:128 * h + 128] = sh
            m = jnp.max(sh, axis=0, keepdims=True)
            mb[8 * j:8 * j + 8, 128 * h:128 * h + 128] = jnp.broadcast_to(m, (8, 128))

    def E_stage(j, u):
        s_, g = unit(u)
        ps, rs = [], []
        for h in range(4):
            m = mb[8 * j:8 * j + 8, 128 * h:128 * h + 128]
            l = None
            pt = []
            for i in range(j + 1):
                r0 = OFF[j] + 128 * i
                s = sb[r0:r0 + 128, 128 * h:128 * h + 128]
                p = jnp.exp2(s.reshape(16, 8, 128) - m[None])
                li = jnp.sum(p, axis=0)
                l = li if l is None else l + li
                pt.append(p.reshape(128, 128).astype(bf16))
            lt = jnp.sum(l, axis=0, keepdims=True)
            rs.append(jnp.broadcast_to(1.0 / lt, (8, 128)) * (1.0 - gate8(g, h)))
            ps.append(pt)
        return ps, rs

    def gate8(g, h):
        return gt[pl.ds(pl.multiple_of(g * 32 + 8 * h, 8), 8), :]

    def V_dots(j, ps, rs):
        outs = []
        for h in range(4):
            acc = None
            for i in range(j + 1):
                vh = i2b(vt[16 * h:16 * h + 16, 128 * i:128 * i + 128])
                d = _dot(vh, ps[h][i])
                acc = d if acc is None else acc + d
            outs.append((acc.reshape(4, 8, 128) * rs[h][None]).reshape(32, 128))
        return jnp.concatenate(outs, axis=0)

    def M_read(u):
        s, g = unit(u)
        mtb = mt[g].astype(bf16)
        nd = _dot(mtb, i2b(pq[u % 4]))
        outs = []
        for h in range(4):
            den = jnp.broadcast_to(nd[128 + h:129 + h], (8, 512)) + 1e-6
            c = jnp.concatenate([gate8(g, h)] * 4, axis=1) / den
            outs.append((nd[32 * h:32 * h + 32].reshape(4, 8, 512) * c[None]).reshape(32, 512))
        return jnp.concatenate(outs, axis=0)

    def V_finish(u, adots, amem):
        s, g = unit(u)
        o = jnp.concatenate(adots, axis=1)
        if amem is not None:
            o = o + amem
        ob[pl.ds(pl.multiple_of(s * 256, 256), 256), col(g)] = b2i(o.astype(bf16).T)

    def M_update(u, first_seg):
        s, g = unit(u)
        ones = jnp.full((8, 512), 0x3F803F80, i32)
        lhs = i2b(jnp.concatenate([vt[...], ones], axis=0))
        upd = _dot(lhs, i2b(pk[u % 4]))
        r = lax.broadcasted_iota(i32, (144, 128), 0)
        c = lax.broadcasted_iota(i32, (144, 128), 1)
        rh = jnp.where(r < 128, r // 32, r - 128)
        upd = jnp.where(rh == c // 32, upd, 0.0)
        if first_seg:
            mt[g] = upd
        else:
            mt[g] = mt[g] + upd

    def D2(v):
        s, c = unit(v)
        o = i2b(ob[pl.ds(pl.multiple_of(s * 256, 256), 256), :])
        y = _dot(o, wo[:, col(c)])
        rows = pl.ds(pl.multiple_of(s * L, L), L)
        xf[rows, col(c)] = xf[rows, col(c)] + y

    def a_iter(t, rep, on, first_seg=False, order="order1"):
        adots = [None] * 4
        pr = [None] * 4
        amem = None
        for tok in cfg[order].split():
            k = tok[0]
            if k not in on:
                continue
            if k == "V":
                adots[int(tok[1])] = V_dots(int(tok[1]), *pr[int(tok[1])])
            elif k == "E":
                pr[int(tok[1])] = E_stage(int(tok[1]), t)
            elif k == "S":
                S_stage(int(tok[1]))
            elif k == "D":
                D2(t - 8)
            elif k == "X":
                XN(jnp.minimum(t + 10, 31), rep)
            elif k == "N":
                LNLN(jnp.maximum(t - 16, 0))
            elif k == "R":
                if not first_seg:
                    amem = M_read(t)
            elif k == "F":
                V_finish(t, adots, amem)
            elif k == "U":
                M_update(t, first_seg)
            elif k == "Q":
                D1q(t + 2)
            elif k == "K":
                D1k(t + 2)
            elif k == "W":
                D1v(t + 1)

    def B1(i, half):
        lhs = i2b(y1[pl.ds(pl.multiple_of(i * (BM // 2), BM // 2), BM // 2), :])
        cols = slice(512 * half, 512 * half + 512)
        hb[pl.ds(pl.multiple_of(i * BM + 8, 8), BM), cols] = _gelu(_dot(lhs, w1[:, cols]))

    def shifted(r0):
        win_ = hb[pl.ds(pl.multiple_of(r0, 8), 144), :]
        parts = []
        for gi, sh in enumerate((-1, 1, -2, 2)):
            parts.append(win_[8 + sh:8 + sh + 128, 256 * gi:256 * gi + 256])
        return jnp.concatenate(parts, axis=1).astype(bf16)

    def bb_body(i, rep):
        rows = [pl.multiple_of(i * BM + 128 * a, 128) for a in range(2)]
        x1 = [zf[pl.ds(r, 128), :] + _dot(shifted(r), w2[...]) for r in rows]
        y2 = [_ln(v).astype(bf16) for v in x1]
        gg = [_gelu(_dot(y2[a], w3[...])).astype(bf16) for a in range(2)]
        for a in range(2):
            r = rows[a]
            xo = xf[pl.ds(r, 128), :] + x1[a] + _dot(gg[a], w4[...])
            xf[pl.ds(r, 128), :] = xo
            xio[pl.ds(r, 128), :] = xo.astype(bf16)

        @pl.when(rep == 1)
        def _():
            o_copy(i).start()
        return rep

    ALL = "VESDXNRFUQKW"

    def l1(t, rep):
        for tt, wi in ((2, 0), (4, 1), (6, 2)):
            @pl.when((rep == 0) & (t == tt))
            def _():
                w_copy(wi).start()
        for tt, q in ((2, 2), (4, 3)):
            @pl.when((rep == 0) & (t == tt))
            def _():
                for m in range(3):
                    qkv_copy(m, q).wait()

        @pl.when((rep == 0) & (t == 6))
        def _():
            x_copy(2).wait()
        a_iter(t, rep, "VESXRFUQKW", first_seg=True)
        return rep

    def l2(t, rep):
        for tt, wi in ((11, 3), (16, 4)):
            @pl.when((rep == 0) & (t == tt))
            def _():
                w_copy(wi).start()

        @pl.when((rep == 0) & (t == 14))
        def _():
            x_copy(3).wait()
        a_iter(t, rep, ALL, order="order2")
        return rep

    if cfg["mode"] == "l2":
        lax.fori_loop(8, 30, l2, 0)
        return
    if cfg["mode"] == "l1":
        lax.fori_loop(0, 8, l1, 0)
        return
    if cfg["mode"] == "bb":
        lax.fori_loop(0, NB, bb_body, 0)
        return

    def rep_body(rep, c):
        with scope("z_xn0"):
            def xn0(c_, carry):
                @pl.when(rep == 0)
                def _():
                    x0_copy(c_).wait()

                @pl.when((rep == 0) & (c_ == 1))
                def _():
                    x_copy(1).start()
                    qkv_copy(2, 0).start()
                XN(c_, rep, 128)
                return carry
            lax.fori_loop(0, 4, xn0, 0)

            @pl.when(rep == 0)
            def _():
                b_copy.wait()
                hr = lax.broadcasted_iota(i32, (H * 8, H), 0) // 8
                hc = lax.broadcasted_iota(i32, (H * 8, H), 1)
                bsel = jnp.sum(jnp.where(hr == hc, bt[...].astype(f32), 0.0), axis=1, keepdims=True)
                gt[...] = jnp.broadcast_to(jax.nn.sigmoid(bsel), (H * 8, 128))

        with scope("z_apro"):
            @pl.when(rep == 0)
            def _():
                qkv_copy(0, 0).wait()
                qkv_copy(1, 0).wait()
            a_iter(-2, rep, "QK")

            @pl.when(rep == 0)
            def _():
                x_copy(1).wait()
                qkv_copy(2, 0).wait()
                for m in range(3):
                    qkv_copy(m, 1).start()
            XN(8, rep)
            XN(9, rep)
            a_iter(-1, rep, "SWQK")

            @pl.when(rep == 0)
            def _():
                for m in range(3):
                    qkv_copy(m, 1).wait()
                for q in (2, 3):
                    for m in range(3):
                        qkv_copy(m, q).start()
                x_copy(2).start()
                x_copy(3).start()

        with scope("z_l1"):
            lax.fori_loop(0, 8, l1, rep)

        @pl.when(rep == 0)
        def _():
            w_copy(0).wait()

        with scope("z_l2"):
            lax.fori_loop(8, 30, l2, rep)
        with scope("z_aepi"):
            a_iter(30, rep, "VESDNRFW", order="order3")
            a_iter(31, rep, "VEDNRF", order="order3")

        @pl.when(rep == 0)
        def _():
            for i in range(1, 5):
                w_copy(i).wait()

        def t1(i, c):
            for tok in cfg["order4"].split():
                if tok[0] == "D":
                    D2(24 + 2 * i + int(tok[1]))
                elif tok[0] == "N":
                    LNLN(8 + i, 128)
                else:
                    B1(i, int(tok[1]))
            return c

        def t2(i, c):
            for tok in cfg["order5"].split():
                if tok[0] == "N":
                    LNLN(jnp.minimum(12 + 2 * (i - 4) + int(tok[1]), 15), 128)
                else:
                    B1(i, int(tok[1]))
            return c
        with scope("z_t1"):
            lax.fori_loop(0, 4, t1, 0)
        with scope("z_t2"):
            lax.fori_loop(4, 8, t2, 0)
        if cfg["mode"] != "A":
            with scope("z_bb"):
                lax.fori_loop(0, NB, bb_body, rep)
        return c

    lax.fori_loop(0, 2, rep_body, 0)
    with scope("z_owait"):
        for i in range(NB):
            o_copy(i).wait()


def build(cfg, name="infini_mixer"):
    vm = pltpu.VMEM
    scratch = [
        vm((S_LEN, D), bf16),
        vm((D, D), bf16), vm((D, D), bf16), vm((D, D), bf16), vm((D, D), bf16),
        vm((D, D), bf16), vm((D, D), bf16), vm((D, F), bf16), vm((F, D), bf16),
        vm((S_LEN, D), f32),
        vm((S_LEN, D), f32),
        vm((S_LEN // 2, D), i32),
        vm((S_LEN // 2, D), i32),
        vm((64, 512), i32), vm((256, 128), i32),
        vm((4, 64, 512), i32), vm((4, 256, 128), i32),
        vm((64, 512), i32),
        vm((1280, 512), f32), vm((32, 512), f32),
        vm((S_LEN // 2, D), i32),
        vm((G, 144, 128), f32),
        vm((S_LEN + 16, D), f32),
        vm((H * 8, 128), f32), vm((1, H), bf16),
        pltpu.SemaphoreType.DMA((4,)), pltpu.SemaphoreType.DMA((3, 4)),
        pltpu.SemaphoreType.DMA((5,)), pltpu.SemaphoreType.DMA((NB,)), pltpu.SemaphoreType.DMA(()),
        pltpu.SemaphoreType.DMA((4,)),
    ]
    any_spec = pl.BlockSpec(memory_space=pl.ANY)
    return pl.pallas_call(
        functools.partial(_kernel, cfg=cfg),
        out_shape=jax.ShapeDtypeStruct((S_LEN, D), bf16),
        in_specs=[any_spec] * 10,
        out_specs=any_spec,
        scratch_shapes=scratch,
        compiler_params=pltpu.CompilerParams(vmem_limit_bytes=110 * 2 ** 20),
        name=name,
    )


def make_kernel(cfg, name="infini_mixer"):
    def kernel(A_x, A_wq, A_wk, A_wv, A_wo, A_beta, B_x, B_w1, B_w2, B_w3, B_w4):
        beta = A_beta.reshape(1, H)
        out = build(cfg, name)(A_x.reshape(S_LEN, D), A_wq, A_wk, A_wv, A_wo, beta, B_w1, B_w2, B_w3, B_w4)
        return out.reshape(1, S_LEN, D)
    return jax.jit(kernel)


pallas_interleave_layers__memory_aug_infini_attn__mixer_s_mlp__prompt_kernel = make_kernel(CFG)
```

```python
import functools
import math

import numpy as np
import jax
import jax.numpy as jnp
from jax import lax
import jax.experimental.pallas as pl
import jax.experimental.pallas.tpu as pltpu

S_LEN = 2048
D = 1024
F = 3584
H = 32
DH = 32
NSEG = 4
L = 512
G = 8
NU = NSEG * G
OFF = (0, 128, 384, 768)
EPS = 1e-5
QSCALE = float(DH ** -0.5 * math.log2(math.e))
NEG = -1e30
BM = 256
NB = S_LEN // BM

f32 = jnp.float32
bf16 = jnp.bfloat16
i32 = jnp.int32
NT = (((1,), (1,)), ((), ()))

CFG = dict(
    order1="R E0 V0 U N E1 V1 E2 S0 S2 E3 V2 S3 V3 F S1 Q W D X K",
    order2="E0 E3 E2 S3 V0 E1 S0 S1 V1 S2 R K V3 V2 U W N Q X F D",
    order3="N E1 S1 V1 E3 X E0 S0 V3 E2 S3 S2 V2 R K V0 U F W D Q",
    order4="B1 D0 N D1 B0",
    order5="B0 N0 B1 N1",
    scopes=False,
)


def i2b(x):
    return pltpu.bitcast(x, bf16)


def b2i(x):
    return pltpu.bitcast(x, i32)


def _ln(x):
    m = jnp.mean(x, axis=-1, keepdims=True)
    d = x - m
    v = jnp.mean(d * d, axis=-1, keepdims=True)
    return d * lax.rsqrt(v + EPS)


def _ln2(x):
    m = jnp.mean(x, axis=-1, keepdims=True)
    d = x - m
    v = jnp.mean(d * d, axis=-1, keepdims=True)
    r = lax.rsqrt(v + EPS)
    r2 = r * lax.rsqrt(v * r * r + EPS)
    return d * r, d * r2


def _gelu(x):
    c0 = math.sqrt(2.0 / math.pi)
    c1 = c0 * 0.044715
    return (0.5 * x) * (1.0 + jnp.tanh(x * (c0 + c1 * (x * x))))


def _phi(t):
    return jnp.where(t > 0, t + 1.0, jnp.exp(t))


def _dot(a, b):
    return jnp.dot(a, b, preferred_element_type=f32)


class _NoScope:
    def __enter__(self):
        return self

    def __exit__(self, *a):
        return False


def _kernel(x_hbm, wq_hbm, wk_hbm, wv_hbm, wo_hbm, beta_hbm, w1_hbm, w2_hbm, w3_hbm, w4_hbm,
            out_hbm,
            xio, wq, wk, wv, wo, w1, w2, w3, w4,
            xf, zf, xn, y1, qs, kb, pq, pk, vt, sb, mb, ob, mt, hb, gt, bt,
            sem_x, sem_q, sem_w, sem_o, sem_b, sem_x0, *, cfg):
    scope = jax.named_scope if cfg["scopes"] else (lambda name: _NoScope())
    wlate = [(wo_hbm, wo), (w1_hbm, w1), (w2_hbm, w2), (w3_hbm, w3), (w4_hbm, w4)]
    wqkv = [(wq_hbm, wq), (wk_hbm, wk), (wv_hbm, wv)]

    def w_copy(i):
        return pltpu.make_async_copy(wlate[i][0], wlate[i][1], sem_w.at[i])

    def qkv_copy(m, q):
        cols = pl.ds(256 * q, 256)
        return pltpu.make_async_copy(wqkv[m][0].at[:, cols], wqkv[m][1].at[:, cols], sem_q.at[m, q])

    def x_copy(i):
        return pltpu.make_async_copy(x_hbm.at[pl.ds(i * L, L)], xio.at[pl.ds(i * L, L)], sem_x.at[i])

    def x0_copy(i):
        r = pl.ds(pl.multiple_of(i * 128, 128), 128)
        return pltpu.make_async_copy(x_hbm.at[r], xio.at[r], sem_x0.at[i])

    def o_copy(i):
        r = pl.multiple_of(i * BM, BM)
        return pltpu.make_async_copy(xio.at[pl.ds(r, BM)], out_hbm.at[pl.ds(r, BM)], sem_o.at[i])

    b_copy = pltpu.make_async_copy(beta_hbm, bt, sem_b)
    for i in range(4):
        x0_copy(i).start()
    qkv_copy(0, 0).start()
    qkv_copy(1, 0).start()
    b_copy.start()
    hb[0:8, :] = jnp.zeros((8, D), f32)
    hb[8 + S_LEN:16 + S_LEN, :] = jnp.zeros((8, D), f32)

    def unit(u):
        return u // G, u % G

    def xs_of(s):
        return i2b(xn[pl.ds(pl.multiple_of(s * (L // 2), L // 2), L // 2), :])

    def col(g):
        return pl.ds(pl.multiple_of(g * 128, 128), 128)

    def rows64(c):
        return pl.ds(pl.multiple_of(c * 64, 64), 64), pl.ds(pl.multiple_of(c * 32, 32), 32)

    def rowsn(c, n):
        return pl.ds(pl.multiple_of(c * n, n), n), pl.ds(pl.multiple_of(c * (n // 2), n // 2), n // 2)

    def XN(c, rep, n=64):
        r, rp = rowsn(c, n)
        x = jnp.where(rep == 0, xio[r, :].astype(f32), xf[r, :])
        xf[r, :] = x
        xn[rp, :] = b2i(_ln(x).astype(bf16))

    def LNLN(c, n=64):
        r, rp = rowsn(c, n)
        z, y = _ln2(xf[r, :])
        zf[r, :] = z
        y1[rp, :] = b2i(y.astype(bf16))

    def D1q(u):
        s, g = unit(u)
        q = _dot(xs_of(s), wq[:, col(g)])
        qs[...] = b2i((q * QSCALE).astype(bf16).T)
        pq[u % 4] = b2i(_phi(q).astype(bf16).T)

    def D1k(u):
        s, g = unit(u)
        k = _dot(xs_of(s), wk[:, col(g)])
        kb[...] = b2i(k.astype(bf16))
        pk[u % 4] = b2i(_phi(k).astype(bf16))

    def D1v(u):
        s, g = unit(u)
        v = _dot(xs_of(s), wv[:, col(g)])
        vt[...] = b2i(v.astype(bf16).T)

    def S_stage(j):
        n = 128 * j + 64
        lane = lax.broadcasted_iota(i32, (64, 128), 1)
        rr = lax.broadcasted_iota(i32, (64, 128), 0)
        valid_lo = rr <= lane
        valid_hi = rr + 64 <= lane
        qj = qs[:, 128 * j:128 * j + 128]
        z16 = jnp.zeros((16, 128), i32)
        hrows = [qj[16 * h:16 * h + 16] for h in range(4)]
        qst = jnp.concatenate(
            [jnp.concatenate([hrows[h] if r == h else z16 for r in range(4)], axis=0) for h in range(4)], axis=1)
        sT = _dot(i2b(kb[:n // 2, :]), i2b(qst))
        upper = lane[:16] >= 64
        prs = []
        for p in range(2):
            ra = jnp.where(upper, hrows[2 * p], 0)
            rb = jnp.where(upper, 0, pltpu.roll(hrows[2 * p + 1], 64, 1))
            prs.append(jnp.concatenate([(ra, rb)[r % 2] if r // 2 == p else z16 for r in range(4)], axis=0))
        sP = _dot(i2b(kb[n // 2:n // 2 + 32, :]), i2b(jnp.concatenate(prs, axis=1)))
        for h in range(4):
            sh = sT[:, 128 * h:128 * h + 128]
            hi = sP[:, 128 * (h // 2):128 * (h // 2) + 128]
            if h % 2:
                hi = pltpu.roll(hi, 64, 1)
            parts = [sh[:128 * j]] if j else []
            parts += [jnp.where(valid_lo, sh[128 * j:], NEG), jnp.where(valid_hi, hi, NEG)]
            sh = jnp.concatenate(parts, axis=0)
            sb[OFF[j]:OFF[j] + n + 64, 128 * h:128 * h + 128] = sh
            m = jnp.max(sh, axis=0, keepdims=True)
            mb[8 * j:8 * j + 8, 128 * h:128 * h + 128] = jnp.broadcast_to(m, (8, 128))

    def E_stage(j, u):
        s_, g = unit(u)
        ps, rs = [], []
        for h in range(4):
            m = mb[8 * j:8 * j + 8, 128 * h:128 * h + 128]
            l = None
            pt = []
            for i in range(j + 1):
                r0 = OFF[j] + 128 * i
                s = sb[r0:r0 + 128, 128 * h:128 * h + 128]
                p = jnp.exp2(s.reshape(16, 8, 128) - m[None])
                li = jnp.sum(p, axis=0)
                l = li if l is None else l + li
                pt.append(p.reshape(128, 128).astype(bf16))
            lt = jnp.sum(l, axis=0, keepdims=True)
            rs.append(jnp.broadcast_to(1.0 / lt, (8, 128)) * (1.0 - gate8(g, h)))
            ps.append(pt)
        return ps, rs

    def gate8(g, h):
        return gt[pl.ds(pl.multiple_of(g * 32 + 8 * h, 8), 8), :]

    def V_dots(j, ps, rs):
        outs = []
        for h in range(4):
            acc = None
            for i in range(j + 1):
                vh = i2b(vt[16 * h:16 * h + 16, 128 * i:128 * i + 128])
                d = _dot(vh, ps[h][i])
                acc = d if acc is None else acc + d
            outs.append((acc.reshape(4, 8, 128) * rs[h][None]).reshape(32, 128))
        return jnp.concatenate(outs, axis=0)

    def M_read(u):
        s, g = unit(u)
        mtb = mt[g].astype(bf16)
        nd = _dot(mtb, i2b(pq[u % 4]))
        outs = []
        for h in range(4):
            den = jnp.broadcast_to(nd[128 + h:129 + h], (8, 512)) + 1e-6
            c = jnp.concatenate([gate8(g, h)] * 4, axis=1) / den
            outs.append((nd[32 * h:32 * h + 32].reshape(4, 8, 512) * c[None]).reshape(32, 512))
        return jnp.concatenate(outs, axis=0)

    def V_finish(u, adots, amem):
        s, g = unit(u)
        o = jnp.concatenate(adots, axis=1)
        if amem is not None:
            o = o + amem
        ob[pl.ds(pl.multiple_of(s * 256, 256), 256), col(g)] = b2i(o.astype(bf16).T)

    def M_update(u, first_seg):
        s, g = unit(u)
        ones = jnp.full((8, 512), 0x3F803F80, i32)
        lhs = i2b(jnp.concatenate([vt[...], ones], axis=0))
        upd = _dot(lhs, i2b(pk[u % 4]))
        r = lax.broadcasted_iota(i32, (144, 128), 0)
        c = lax.broadcasted_iota(i32, (144, 128), 1)
        rh = jnp.where(r < 128, r // 32, r - 128)
        upd = jnp.where(rh == c // 32, upd, 0.0)
        if first_seg:
            mt[g] = upd
        else:
            mt[g] = mt[g] + upd

    def D2(v):
        s, c = unit(v)
        o = i2b(ob[pl.ds(pl.multiple_of(s * 256, 256), 256), :])
        y = _dot(o, wo[:, col(c)])
        rows = pl.ds(pl.multiple_of(s * L, L), L)
        xf[rows, col(c)] = xf[rows, col(c)] + y

    def a_iter(t, rep, on, first_seg=False, order="order1"):
        adots = [None] * 4
        pr = [None] * 4
        amem = None
        for tok in cfg[order].split():
            k = tok[0]
            if k not in on:
                continue
            if k == "V":
                adots[int(tok[1])] = V_dots(int(tok[1]), *pr[int(tok[1])])
            elif k == "E":
                pr[int(tok[1])] = E_stage(int(tok[1]), t)
            elif k == "S":
                S_stage(int(tok[1]))
            elif k == "D":
                D2(t - 8)
            elif k == "X":
                XN(jnp.minimum(t + 10, 31), rep)
            elif k == "N":
                LNLN(jnp.maximum(t - 16, 0))
            elif k == "R":
                if not first_seg:
                    amem = M_read(t)
            elif k == "F":
                V_finish(t, adots, amem)
            elif k == "U":
                M_update(t, first_seg)
            elif k == "Q":
                D1q(t + 2)
            elif k == "K":
                D1k(t + 2)
            elif k == "W":
                D1v(t + 1)

    def B1(i, half):
        lhs = i2b(y1[pl.ds(pl.multiple_of(i * (BM // 2), BM // 2), BM // 2), :])
        cols = slice(512 * half, 512 * half + 512)
        hb[pl.ds(pl.multiple_of(i * BM + 8, 8), BM), cols] = _gelu(_dot(lhs, w1[:, cols]))

    def shifted(r0):
        win_ = hb[pl.ds(pl.multiple_of(r0, 8), 144), :]
        parts = []
        for gi, sh in enumerate((-1, 1, -2, 2)):
            parts.append(win_[8 + sh:8 + sh + 128, 256 * gi:256 * gi + 256])
        return jnp.concatenate(parts, axis=1).astype(bf16)

    def bb_body(i, rep):
        rows = [pl.multiple_of(i * BM + 128 * a, 128) for a in range(2)]
        x1 = [zf[pl.ds(r, 128), :] + _dot(shifted(r), w2[...]) for r in rows]
        y2 = [_ln(v).astype(bf16) for v in x1]
        gg = [_gelu(_dot(y2[a], w3[...])).astype(bf16) for a in range(2)]
        for a in range(2):
            r = rows[a]
            xo = xf[pl.ds(r, 128), :] + x1[a] + _dot(gg[a], w4[...])
            xf[pl.ds(r, 128), :] = xo
            xio[pl.ds(r, 128), :] = xo.astype(bf16)

        @pl.when(rep == 1)
        def _():
            o_copy(i).start()
        return rep

    ALL = "VESDXNRFUQKW"

    def l1(t, rep):
        for tt, wi in ((2, 0), (4, 1), (6, 2)):
            @pl.when((rep == 0) & (t == tt))
            def _():
                w_copy(wi).start()
        for tt, q in ((2, 2), (4, 3)):
            @pl.when((rep == 0) & (t == tt))
            def _():
                for m in range(3):
                    qkv_copy(m, q).wait()

        @pl.when((rep == 0) & (t == 6))
        def _():
            x_copy(2).wait()
        a_iter(t, rep, "VESXRFUQKW", first_seg=True)
        return rep

    def l2(t, rep):
        for tt, wi in ((11, 3), (16, 4)):
            @pl.when((rep == 0) & (t == tt))
            def _():
                w_copy(wi).start()

        @pl.when((rep == 0) & (t == 14))
        def _():
            x_copy(3).wait()
        a_iter(t, rep, ALL, order="order2")
        return rep

    def rep_body(rep, c):
        with scope("z_xn0"):
            def xn0(c_, carry):
                @pl.when(rep == 0)
                def _():
                    x0_copy(c_).wait()

                @pl.when((rep == 0) & (c_ == 1))
                def _():
                    x_copy(1).start()
                    qkv_copy(2, 0).start()
                XN(c_, rep, 128)
                return carry
            lax.fori_loop(0, 4, xn0, 0)

            @pl.when(rep == 0)
            def _():
                b_copy.wait()
                hr = lax.broadcasted_iota(i32, (H * 8, H), 0) // 8
                hc = lax.broadcasted_iota(i32, (H * 8, H), 1)
                bsel = jnp.sum(jnp.where(hr == hc, bt[...].astype(f32), 0.0), axis=1, keepdims=True)
                gt[...] = jnp.broadcast_to(jax.nn.sigmoid(bsel), (H * 8, 128))

        with scope("z_apro"):
            @pl.when(rep == 0)
            def _():
                qkv_copy(0, 0).wait()
                qkv_copy(1, 0).wait()
            a_iter(-2, rep, "QK")

            @pl.when(rep == 0)
            def _():
                x_copy(1).wait()
                qkv_copy(2, 0).wait()
                for m in range(3):
                    qkv_copy(m, 1).start()
            XN(8, rep)
            XN(9, rep)
            a_iter(-1, rep, "SWQK")

            @pl.when(rep == 0)
            def _():
                for m in range(3):
                    qkv_copy(m, 1).wait()
                for q in (2, 3):
                    for m in range(3):
                        qkv_copy(m, q).start()
                x_copy(2).start()
                x_copy(3).start()

        with scope("z_l1"):
            lax.fori_loop(0, 8, l1, rep)

        @pl.when(rep == 0)
        def _():
            w_copy(0).wait()

        with scope("z_l2"):
            lax.fori_loop(8, 30, l2, rep)
        with scope("z_aepi"):
            a_iter(30, rep, "VESDNRFW", order="order3")
            a_iter(31, rep, "VEDNRF", order="order3")

        @pl.when(rep == 0)
        def _():
            for i in range(1, 5):
                w_copy(i).wait()

        def t1(i, c):
            for tok in cfg["order4"].split():
                if tok[0] == "D":
                    D2(24 + 2 * i + int(tok[1]))
                elif tok[0] == "N":
                    LNLN(8 + i, 128)
                else:
                    B1(i, int(tok[1]))
            return c

        def t2(i, c):
            for tok in cfg["order5"].split():
                if tok[0] == "N":
                    LNLN(jnp.minimum(12 + 2 * (i - 4) + int(tok[1]), 15), 128)
                else:
                    B1(i, int(tok[1]))
            return c
        with scope("z_t1"):
            lax.fori_loop(0, 4, t1, 0)
        with scope("z_t2"):
            lax.fori_loop(4, 8, t2, 0)
        with scope("z_bb"):
            lax.fori_loop(0, NB, bb_body, rep)
        return c

    lax.fori_loop(0, 2, rep_body, 0)
    with scope("z_owait"):
        for i in range(NB):
            o_copy(i).wait()


def build(cfg, name="infini_mixer"):
    vm = pltpu.VMEM
    scratch = [
        vm((S_LEN, D), bf16),
        vm((D, D), bf16), vm((D, D), bf16), vm((D, D), bf16), vm((D, D), bf16),
        vm((D, D), bf16), vm((D, D), bf16), vm((D, F), bf16), vm((F, D), bf16),
        vm((S_LEN, D), f32),
        vm((S_LEN, D), f32),
        vm((S_LEN // 2, D), i32),
        vm((S_LEN // 2, D), i32),
        vm((64, 512), i32), vm((256, 128), i32),
        vm((4, 64, 512), i32), vm((4, 256, 128), i32),
        vm((64, 512), i32),
        vm((1280, 512), f32), vm((32, 512), f32),
        vm((S_LEN // 2, D), i32),
        vm((G, 144, 128), f32),
        vm((S_LEN + 16, D), f32),
        vm((H * 8, 128), f32), vm((1, H), bf16),
        pltpu.SemaphoreType.DMA((4,)), pltpu.SemaphoreType.DMA((3, 4)),
        pltpu.SemaphoreType.DMA((5,)), pltpu.SemaphoreType.DMA((NB,)), pltpu.SemaphoreType.DMA(()),
        pltpu.SemaphoreType.DMA((4,)),
    ]
    any_spec = pl.BlockSpec(memory_space=pl.ANY)
    return pl.pallas_call(
        functools.partial(_kernel, cfg=cfg),
        out_shape=jax.ShapeDtypeStruct((S_LEN, D), bf16),
        in_specs=[any_spec] * 10,
        out_specs=any_spec,
        scratch_shapes=scratch,
        compiler_params=pltpu.CompilerParams(vmem_limit_bytes=110 * 2 ** 20),
        name=name,
    )


def make_kernel(cfg, name="infini_mixer"):
    def kernel(A_x, A_wq, A_wk, A_wv, A_wo, A_beta, B_x, B_w1, B_w2, B_w3, B_w4):
        beta = A_beta.reshape(1, H)
        out = build(cfg, name)(A_x.reshape(S_LEN, D), A_wq, A_wk, A_wv, A_wo, beta, B_w1, B_w2, B_w3, B_w4)
        return out.reshape(1, S_LEN, D)
    return jax.jit(kernel)


pallas_interleave_layers__memory_aug_infini_attn__mixer_s_mlp__prompt_kernel = make_kernel(CFG)
```
